```python
import os as _os
_os.environ.setdefault("JAX_PLATFORMS", "cpu")
import jax
import jax.numpy as jnp

def _softmax(x, axis=-1):
    return jax.nn.softmax(x, axis=axis)
def _gelu(x):
    return jax.nn.gelu(x, approximate=True)
def _silu(x):
    return jax.nn.silu(x)
def _sigmoid(x):
    return jax.nn.sigmoid(x)
def _layernorm(x, axis=-1, eps=1e-5):
    m = jnp.mean(x, axis=axis, keepdims=True)
    v = jnp.var(x, axis=axis, keepdims=True)
    return (x - m) / jnp.sqrt(v + eps)
def _scatter_add(tgt, idx, src, axis=0):
    return tgt.at[idx].add(src)
def _segment_sum(src, seg, n):
    return jax.ops.segment_sum(src, seg, n)
class _Rng:
    def __init__(self, key):
        self._k = key
    def _next(self):
        self._k, sub = jax.random.split(self._k)
        return sub
    def normal(self, shape):
        return jax.random.normal(self._next(), shape, dtype=jnp.bfloat16)
    def randint(self, lo, hi, shape):
        return jax.random.randint(self._next(), shape, lo, hi, dtype=jnp.int32)
    def uniform(self, shape, lo=0.0, hi=1.0):
        return jax.random.uniform(self._next(), shape, jnp.bfloat16, lo, hi)
    def permutation(self, n):
        return jax.random.permutation(self._next(), n)


kernel_name = 'interleave_layers__mha_block__dense_activation_gelu__prompt'

def setup_inputs():
    _rng = _Rng(jax.random.key(int.from_bytes(__import__("os").urandom(4), "little")))
    _w = (lambda a: (lambda t: t.astype(jnp.bfloat16) if jnp.issubdtype(t.dtype, jnp.floating) else t)(jnp.asarray(a)))
    def _A_setup():
        B, S, D, H = 1, 2048, 512, 32
        return {
            "x": _w((lambda *s: _rng.normal(s) * 0.05)(B, S, D)),
            "wqkv": _w((lambda *s: _rng.normal(s) * 0.05)(D, 3 * D)),
            "wo": _w((lambda *s: _rng.normal(s) * 0.05)(D, D)),
        }
    _A_in = _A_setup()

    def _B_setup():
        B, S, D, F = 1, 2048, 512, 1792
        return {
            "x": _w((lambda *s: _rng.normal(s) * 0.05)(B, S, D)),
            "w1": _w((lambda *s: _rng.normal(s) * 0.4)(D, F) * (D ** -0.5)),
            "b1": _w((lambda *s: _rng.normal(s) * 0.4)(F) * 0.01),
            "w2": _w((lambda *s: _rng.normal(s) * 0.4)(F, D) * (F ** -0.5)),
            "b2": _w((lambda *s: _rng.normal(s) * 0.4)(D) * 0.01),
        }
    _B_in = _B_setup()

    return {
        "A_x": _A_in["x"],
        "A_wqkv": _A_in["wqkv"],
        "A_wo": _A_in["wo"],
        "B_x": _B_in["x"],
        "B_w1": _B_in["w1"],
        "B_b1": _B_in["b1"],
        "B_w2": _B_in["w2"],
        "B_b2": _B_in["b2"],
    }

def reference(A_x, A_wqkv, A_wo, B_x, B_w1, B_b1, B_w2, B_b2):
    def _A_ref(x, wqkv, wo):
        B, S, D = x.shape
        H = 32
        Dh = D // H
        qkv = (lambda x, *d: x.transpose(*d))((x @ wqkv).reshape(B, S, 3, H, Dh), 2, 0, 3, 1, 4)
        q, k, v = qkv[0], qkv[1], qkv[2]
        scores = jnp.einsum("bhqd,bhkd->bhqk", q, k) * (Dh ** -0.5)
        p = _softmax(scores, axis=-1)
        o = jnp.einsum("bhqk,bhkd->bhqd", p, v)
        return (lambda x, *d: x.transpose(*d))(o, 0, 2, 1, 3).reshape(B, S, D) @ wo

    def _B_ref(x, w1, b1, w2, b2):
        h = jnp.einsum("bsd,df->bsf", x, w1) + b1
        h = _gelu(h)
        return jnp.einsum("bsf,fd->bsd", h, w2) + b2

    x = A_x
    x = x + _A_ref(_layernorm(x, axis=-1), A_wqkv, A_wo)
    x = x + _B_ref(_layernorm(x, axis=-1), B_w1, B_b1, B_w2, B_b2)
    x = x + _A_ref(_layernorm(x, axis=-1), A_wqkv, A_wo)
    x = x + _B_ref(_layernorm(x, axis=-1), B_w1, B_b1, B_w2, B_b2)
    return x
```

```python
import jax
import jax.numpy as jnp
from jax import lax
import jax.experimental.pallas as pl
import jax.experimental.pallas.tpu as pltpu

S, D, H, DH, F = 2048, 512, 32, 16, 1792
TR = 256
TQ = 512
KC = 128
NB = S // TQ
NC = S // KC
LAG = 3
VL = 3
NS = (6, 9, 9, 9)
START = 96
MARG = 0
NVM = (max(NS) + 3) // 4
NR = LAG + 2
NPV = 2 * NVM
NZ = 300
LOG2E = 1.4426950408889634
QSCALE = (DH ** -0.5) * LOG2E
SAFE_LOG2 = 60.0
bf16 = jnp.bfloat16
f32 = jnp.float32
u32 = jnp.uint32


def _ln(x):
    m = jnp.mean(x, axis=-1, keepdims=True)
    xc = x - m
    v = jnp.mean(xc * xc, axis=-1, keepdims=True)
    return xc * lax.rsqrt(v + 1e-5)


def _gelu(x):
    c = 0.7978845608028654
    return 0.5 * x * (1.0 + jnp.tanh(c * (x + 0.044715 * (x * x * x))))


def _pack_rows(p):
    r, w = p.shape
    p4 = p.reshape(r // 16, 2, 8, w)
    return pltpu.pack_elementwise([p4[:, 0], p4[:, 1]], packed_dtype=bf16).reshape(r // 2, w).astype(u32)


def _kernel(x_ref, wqkv_ref, wo_ref, w1_ref, b1_ref, w2_ref, b2_ref, o_ref,
            xres, wqt, wvt, k_s, qt_s, vt_s, qf_s, kt_s, ot_s, qm_s, st_s, sc_s, z_s, *bufs):
    ring = bufs[:NR]
    pvb = bufs[NR:NR + NPV]
    kbs = bufs[NR + NPV:]
    wqt[...] = wqkv_ref[:, 0:D].astype(f32).T.astype(bf16)
    wvt[...] = wqkv_ref[:, 2 * D:3 * D].astype(f32).T.astype(bf16)
    qm_s[...] = jnp.zeros_like(qm_s)
    st_s[...] = jnp.zeros_like(st_s)
    for i in range(NZ):
        z_s[i] = 0

    nt = (((1,), (1,)), ((), ()))

    def proj(r0, x):
        xn = _ln(x)
        xb = xn.astype(bf16)
        xi = pltpu.bitcast(_pack_rows(xn), bf16)
        k = jnp.dot(xb, wqkv_ref[:, D:2 * D], preferred_element_type=f32)
        kp = pltpu.bitcast(k.astype(bf16), u32)
        r2 = pl.multiple_of(r0 // 2, TR // 2)
        for g in range(4):
            k_s[g, pl.ds(r2, TR // 2), :] = kp[:, g * 128:(g + 1) * 128]
        kt = k.T.reshape(H, DH, TR)
        kt_s[:, :, pl.ds(r0, TR)] = kt
        q = lax.dot_general(wqt[...], xb, nt, preferred_element_type=f32) * QSCALE
        qt_s[:, pl.ds(r0, TR)] = pltpu.bitcast(q.astype(bf16), u32)
        q3 = q.reshape(H, DH, TR)
        qf_s[:, :, pl.ds(r0, TR)] = q3
        v = lax.dot_general(wvt[...], xi, nt, preferred_element_type=f32)
        vt_s[:, pl.ds(r0, TR)] = pltpu.bitcast(v.astype(bf16), u32)
        st_s[0] = jnp.maximum(st_s[0], jnp.sum(q3 * q3, axis=1))
        st_s[1] = jnp.maximum(st_s[1], jnp.sum(kt * kt, axis=1))
        st_s[2] = jnp.maximum(st_s[2], jnp.max(jnp.abs(v).reshape(DH, H, TR), axis=0))

    def first(r, c):
        r0 = pl.multiple_of(r * TR, TR)
        x = x_ref[pl.ds(r0, TR), :].astype(f32)
        xres[pl.ds(r0, TR), :] = x
        proj(r0, x)
        return c
    lax.fori_loop(0, S // TR, first, 0)

    def set_q(h):
        moff = pl.multiple_of((h % 8) * 8, 8)
        poff = pl.multiple_of(((h + 7) % 8) * 8, 8)
        qm_s[0, pl.ds(poff, 8), :] = jnp.zeros((8, S), u32)
        qm_s[0, pl.ds(moff, 8), :] = qt_s[pl.ds(pl.multiple_of(h * 8, 8), 8), :]

    def head_fast(h, c):
        g = h // 8
        hoff = pl.multiple_of(h * DH, DH)
        h8 = pl.multiple_of(h * 8, 8)
        set_q(h)
        for t in range(NVM):
            for d in range(DH):
                row = jnp.broadcast_to(kt_s[h, pl.ds(d, 1), pl.ds(t * 128, 128)], (128, 128))
                kbs[t][0, d] = row.T
        zc = [0]

        def zero():
            zc[0] += 1
            return z_s[zc[0] - 1]
        o = [jnp.zeros((DH, TQ), f32) for _ in range(NB)]
        l = [[None] * 4 for _ in range(NB)]
        where = {}
        cnt = [0]
        attach = {}
        vdone = {}
        mx = []
        for b in range(NB):
            n = NS[b]
            lst = [(b, ci, (n % 4) * 32 if ci == n // 4 else 0) for ci in range(n // 4, NC)]
            rows = [(x, r) for x in lst for r in range(x[2] // 8, 16)]
            npc = n * 4
            st = START if b == 0 else 0
            npos = len(rows) - (MARG if b == NB - 1 else 0) - st
            for k in range(npc):
                sub, j = divmod(k, 4)
                x, r = rows[st + int((k + 0.5) * npos / npc)]
                attach.setdefault((x, r, j), []).append(sub)
                vdone[(b, sub // 4)] = x
            mx += lst

        def addl(b, j, v):
            l[b][j] = v if l[b][j] is None else l[b][j] + v

        def do_qk(b, ci, r0):
            z = zero()
            kc = pltpu.bitcast(k_s[g + z, pl.ds((ci * KC + r0) // 2, (KC - r0) // 2), :], bf16)
            qm = pltpu.bitcast(qm_s[z, :, pl.ds(b * TQ, TQ)], bf16)
            p = jnp.exp2(jnp.dot(kc, qm, preferred_element_type=f32))
            for r in range(r0 // 8, 16):
                rr = r - r0 // 8
                for j in range(4):
                    addl(b, j, p[8 * rr:8 * rr + 8, 128 * j:128 * j + 128])
                    for sub in attach.get(((b, ci, r0), r, j), []):
                        addl(b, j, do_vpu(b, sub, j))
            if r0:
                pvb[(b * NVM + ci) % NPV][0, pl.ds(r0 // 2, (KC - r0) // 2), :] = _pack_rows(p)
            else:
                r = ring[cnt[0] % NR]
                cnt[0] += 1
                r[0] = _pack_rows(p)
                where[(b, ci)] = r

        def do_vpu(b, sub, j):
            ci, sb = divmod(sub, 4)
            acc = None
            z = zero()
            hq = h + z
            for d in range(DH):
                kbd = kbs[ci][z, d, pl.ds(sb * 32, 32), :]
                qd = qf_s[hq, pl.ds(d, 1), pl.ds(b * TQ + j * 128, 128)]
                t = kbd * qd
                acc = t if acc is None else acc + t
            p = jnp.exp2(acc)
            pvb[(b * NVM + ci) % NPV][0, pl.ds(sb * 16, 16), pl.ds(j * 128, 128)] = _pack_rows(p)
            return jnp.sum(p.reshape(4, 8, 128), axis=0)
        done = [0] * NB

        def do_pv(b, ci):
            z = zero()
            vt = pltpu.bitcast(vt_s[pl.ds(h8, 8), pl.ds(ci * KC, KC)], bf16)
            src = where.pop((b, ci)) if (b, ci) in where else pvb[(b * NVM + ci) % NPV]
            o[b] = o[b] + jnp.dot(vt, pltpu.bitcast(src[z], bf16), preferred_element_type=f32)
            done[b] += 1
            if done[b] == NC:
                lsum = jnp.sum(jnp.concatenate(l[b], axis=-1), axis=0, keepdims=True)
                ot_s[pl.ds(hoff, DH), pl.ds(b * TQ, TQ)] = o[b] * (1.0 / lsum)
        pvq = []
        for i, it in enumerate(mx):
            do_qk(*it)
            if it[2] == 0:
                pvq.append((i + LAG, it[:2]))
            for key, x in vdone.items():
                if x == it:
                    pvq.append((i + VL, key))
            rdy = [x for x in pvq if x[0] <= i]
            pvq = [x for x in pvq if x[0] > i]
            for _, it2 in rdy:
                do_pv(*it2)
        for _, it2 in sorted(pvq):
            do_pv(*it2)
        assert all(d == NC for d in done) and zc[0] <= NZ
        return c

    def head_safe(h, c):
        g = h // 8
        hoff = pl.multiple_of(h * DH, DH)
        h8 = pl.multiple_of(h * 8, 8)
        set_q(h)

        def blk(b, c2):
            q0 = pl.multiple_of(b * TQ, TQ)
            qm = pltpu.bitcast(qm_s[0, :, pl.ds(q0, TQ)], bf16)
            m = jnp.full((8, TQ), -jnp.inf, f32)
            for c0 in range(0, S, 256):
                kc = pltpu.bitcast(k_s[g, pl.ds(c0 // 2, 128), :], bf16)
                s = jnp.dot(kc, qm, preferred_element_type=f32)
                sc_s[pl.ds(c0, 256), :] = s
                m = jnp.maximum(m, jnp.max(s.reshape(32, 8, TQ), axis=0))
            m = jnp.max(m, axis=0, keepdims=True)
            l = jnp.zeros((8, TQ), f32)
            o = jnp.zeros((DH, TQ), f32)
            for c0 in range(0, S, 256):
                p = jnp.exp2(sc_s[pl.ds(c0, 256), :] - m)
                l = l + jnp.sum(p.reshape(32, 8, TQ), axis=0)
                vt = pltpu.bitcast(vt_s[pl.ds(h8, 8), pl.ds(c0, 256)], bf16)
                o = o + jnp.dot(vt, pltpu.bitcast(_pack_rows(p), bf16), preferred_element_type=f32)
            ot_s[pl.ds(hoff, DH), pl.ds(q0, TQ)] = o * (1.0 / jnp.sum(l, axis=0, keepdims=True))
            return c2
        lax.fori_loop(0, NB, blk, 0)
        return c

    def attention():
        qn = jnp.max(st_s[0], axis=1, keepdims=True)
        kn = jnp.max(st_s[1], axis=1, keepdims=True)
        bound2 = jnp.max(qn * kn) * 1.05
        vmax = jnp.max(st_s[2])
        st_s[...] = jnp.zeros_like(st_s)
        ok = jnp.logical_and(bound2 <= SAFE_LOG2 * SAFE_LOG2,
                             jnp.logical_and(vmax <= 2.0 ** 40, vmax >= 2.0 ** -30))

        @pl.when(ok)
        def _():
            lax.fori_loop(0, H, head_fast, 0)

        @pl.when(jnp.logical_not(ok))
        def _():
            lax.fori_loop(0, H, head_safe, 0)

    def dense(last):
        def body(r, c):
            r0 = pl.multiple_of(r * TR, TR)
            o = ot_s[:, pl.ds(r0, TR)].T.astype(bf16)
            x = xres[pl.ds(r0, TR), :] + jnp.dot(o, wo_ref[...], preferred_element_type=f32)
            xn = _ln(x).astype(bf16)
            hh = jnp.dot(xn, w1_ref[...], preferred_element_type=f32) + b1_ref[...].astype(f32)
            hh = _gelu(hh).astype(bf16)
            x = x + jnp.dot(hh, w2_ref[...], preferred_element_type=f32) + b2_ref[...].astype(f32)
            if last:
                o_ref[pl.ds(r0, TR), :] = x.astype(o_ref.dtype)
            else:
                xres[pl.ds(r0, TR), :] = x
                proj(r0, x)
            return c
        lax.fori_loop(0, S // TR, body, 0)

    def layer(i, c):
        attention()

        @pl.when(i == 0)
        def _():
            dense(False)

        @pl.when(i == 1)
        def _():
            dense(True)
        return c
    lax.fori_loop(0, 2, layer, 0)


@jax.jit
def pallas_interleave_layers__mha_block__dense_activation_gelu__prompt_kernel(A_x, A_wqkv, A_wo, B_x, B_w1, B_b1, B_w2, B_b2):
    x = A_x.reshape(S, D)
    out = pl.pallas_call(
        _kernel,
        out_shape=jax.ShapeDtypeStruct((S, D), bf16),
        scratch_shapes=[
            pltpu.VMEM((S, D), f32),
            pltpu.VMEM((D, D), bf16),
            pltpu.VMEM((D, D), bf16),
            pltpu.VMEM((4, S // 2, 128), u32),
            pltpu.VMEM((D // 2, S), u32),
            pltpu.VMEM((D // 2, S), u32),
            pltpu.VMEM((H, DH, S), f32),
            pltpu.VMEM((H, DH, S), f32),
            pltpu.VMEM((D, S), f32),
            pltpu.VMEM((1, 64, S), u32),
            pltpu.VMEM((3, H, TR), f32),
            pltpu.VMEM((S, TQ), f32),
            pltpu.SMEM((NZ,), jnp.int32),
        ] + [pltpu.VMEM((1, 64, TQ), u32) for _ in range(NR + NPV)]
          + [pltpu.VMEM((1, DH, 128, 128), f32) for _ in range(NVM)],
        compiler_params=pltpu.CompilerParams(vmem_limit_bytes=100 * 2 ** 20),
    )(x, A_wqkv, A_wo, B_w1, B_b1.reshape(1, F), B_w2, B_b2.reshape(1, D))
    return out.reshape(1, S, D)
```

```python
import jax
import jax.numpy as jnp
from jax import lax
import jax.experimental.pallas as pl
import jax.experimental.pallas.tpu as pltpu

S, D, H, DH, F = 2048, 512, 32, 16, 1792
TR = 128
NT = 4
TI = TR * NT
TQ = 512
KC = 128
NB = S // TQ
NC = S // KC
LAG = 4
NS = (5, 9, 9, 9)
START = 16
PVM = 2
NPF = 3


def _groups(first, n):
    out = [(first + i, 32) for i in range(int(n))]
    if n != int(n):
        out.append((first + int(n), 16))
    return out


SUBS = [_groups(4, n) for n in NS]
SUBS[0] = _groups(0, NPF) + SUBS[0]
NVM = 4
NR = 16
NL = 36
NZ = 600
LOG2E = 1.4426950408889634
QSCALE = (DH ** -0.5) * LOG2E
SAFE_LOG2 = 60.0
bf16 = jnp.bfloat16
f32 = jnp.float32
u32 = jnp.uint32


def _ln(x):
    m = jnp.mean(x, axis=-1, keepdims=True)
    xc = x - m
    v = jnp.mean(xc * xc, axis=-1, keepdims=True)
    return xc * lax.rsqrt(v + 1e-5)


def _gelu(x):
    c = 0.7978845608028654
    return 0.5 * x * (1.0 + jnp.tanh(c * (x + 0.044715 * (x * x * x))))


def _pack_rows(p):
    r, w = p.shape
    p4 = p.reshape(r // 16, 2, 8, w)
    return pltpu.pack_elementwise([p4[:, 0], p4[:, 1]], packed_dtype=bf16).reshape(r // 2, w).astype(u32)


def _plan():
    nrows = sum(NC * 16 - sum(r // 8 for _, r in x) for x in SUBS)
    pieces = [(b, c, a, j) for b in range(NB) for c, r in SUBS[b] for a in range(r // 16) for j in range(4)]
    pos = {pc: START + int((k + 0.5) * (nrows - START) / len(pieces)) for k, pc in enumerate(pieces)}
    order = []
    row = 0
    for b in range(NB):
        mixed = list(SUBS[b])
        pure = [c for c in range(NC) if c not in dict(mixed)]
        while mixed or pure:
            if mixed and (not pure or row + (LAG - PVM) * 14 > pos[(b, mixed[0][0], mixed[0][1] // 16 - 1, 3)]):
                order.append((b,) + mixed.pop(0))
            else:
                order.append((b, pure.pop(0), 0))
            row += 16 - order[-1][2] // 8
    rows = [(i, r) for i, x in enumerate(order) for r in range(16 - x[2] // 8)]
    attach = {}
    foreign = {(b, j): [] for b in range(NB) for j in range(4)}
    for (pb, c, a, j), p in pos.items():
        i, r = rows[p]
        attach.setdefault((i, r, j), []).append((pb, c, a))
        if pb != order[i][0]:
            foreign[(pb, j)].append(c * 2 + a)
    return order, attach, foreign


def _kernel(x_hbm, wqkv_hbm, wo_hbm, w1_hbm, b1_ref, w2_hbm, b2_ref, o_hbm,
            x_ref, wqkv_ref, wo_ref, w1_ref, w2_ref, sem_x, sem_w, sem_o,
            xres, wqt, wvt, k_s, qt_s, vt_s, qf_s, kt_s, ot_s, qm_s, st_s, sc_s, zv_s, z_s, *bufs):
    ring = bufs[:NR]
    kbs = bufs[NR:NR + NVM]
    lacc = bufs[NR + NVM:]

    def x_copy(r):
        rows = pl.ds(pl.multiple_of(r * TI, TI), TI)
        return pltpu.make_async_copy(x_hbm.at[rows], x_ref.at[rows], sem_x.at[r])

    def o_copy(r):
        rows = pl.ds(pl.multiple_of(r * TI, TI), TI)
        return pltpu.make_async_copy(x_ref.at[rows], o_hbm.at[rows], sem_o.at[r])
    w_copies = [pltpu.make_async_copy(a, b, sem_w.at[i]) for i, (a, b) in enumerate(
        [(wqkv_hbm, wqkv_ref), (wo_hbm, wo_ref), (w1_hbm, w1_ref), (w2_hbm, w2_ref)])]
    w_copies[0].start()
    for r in range(S // TI):
        x_copy(r).start()
    for cp in w_copies[1:]:
        cp.start()
    qm_s[...] = jnp.zeros_like(qm_s)
    st_s[...] = jnp.zeros_like(st_s)
    zv_s[...] = jnp.zeros_like(zv_s)
    kt_s[0, 0] = jnp.zeros((DH, 128), f32)
    for buf in ring[NR - LAG:]:
        buf[...] = jnp.zeros_like(buf)
    lacc[NB - 1][...] = jnp.ones_like(lacc[NB - 1])
    for i in range(NZ):
        z_s[i] = 0
    w_copies[0].wait()
    wqt[...] = wqkv_ref[:, 0:D].astype(f32).T.astype(bf16)
    wvt[...] = wqkv_ref[:, 2 * D:3 * D].astype(f32).T.astype(bf16)

    nt = (((1,), (1,)), ((), ()))

    def proj(r0, x):
        xn = _ln(x)
        xb = xn.astype(bf16)
        xi = pltpu.bitcast(_pack_rows(xn), bf16)
        k = jnp.dot(xb, wqkv_ref[:, D:2 * D], preferred_element_type=f32)
        kp = pltpu.bitcast(k.astype(bf16), u32)
        r2 = pl.multiple_of(r0 // 2, TR // 2)
        for g in range(4):
            k_s[g, pl.ds(r2, TR // 2), :] = kp[:, g * 128:(g + 1) * 128]
        kt = k.T.reshape(H, DH, TR)
        q = lax.dot_general(wqt[...], xb, nt, preferred_element_type=f32) * QSCALE
        qt_s[:, pl.ds(r0, TR)] = pltpu.bitcast(q.astype(bf16), u32)
        q3 = q.reshape(H, DH, TR)
        qf_s[:, :, pl.ds(r0, TR)] = q3
        v = lax.dot_general(wvt[...], xi, nt, preferred_element_type=f32)
        vt_s[:, pl.ds(r0, TR)] = pltpu.bitcast(v.astype(bf16), u32)
        st_s[0] = jnp.maximum(st_s[0], jnp.sum(q3 * q3, axis=1))
        st_s[1] = jnp.maximum(st_s[1], jnp.sum(kt * kt, axis=1))
        st_s[2] = jnp.maximum(st_s[2], jnp.max(jnp.abs(v).reshape(DH, H, TR), axis=0))

        return [k[c0:c0 + 32] for c0 in range(0, TR, KC)]

    def prep(h, t):
        for d in range(DH):
            row = jnp.broadcast_to(kt_s[t, h, pl.ds(d, 1), :], (128, 128))
            kbs[t][0, d] = row.T

    def put_kt(r, heads):
        kt_s[r] = jnp.concatenate(heads, axis=0).T.reshape(H, DH, 128)

    def first(r, c):
        x_copy(r).wait()
        prep(0, 0)
        kh = []
        for t in range(NT):
            r0 = pl.multiple_of(r * TI + t * TR, TR)
            x = x_ref[pl.ds(r0, TR), :].astype(f32)
            xres[pl.ds(r0, TR), :] = x
            kh += proj(r0, x)
        put_kt(r, kh)
        return c
    lax.fori_loop(0, S // TI, first, 0)

    def set_q(h):
        moff = pl.multiple_of((h % 8) * 8, 8)
        poff = pl.multiple_of(((h + 7) % 8) * 8, 8)
        qm_s[0, pl.ds(poff, 8), :] = jnp.zeros((8, S), u32)
        qm_s[0, pl.ds(moff, 8), :] = qt_s[pl.ds(pl.multiple_of(h * 8, 8), 8), :]

    order, attach, foreign = _plan()
    no = len(order)
    bufof = {x[:2]: ring[i % NR] for i, x in enumerate(order)}

    def head_fast(h, o_prev, main=True):
        g = h // 8
        hp = jnp.maximum(h - 1, 0)
        hpo = jnp.where(h > 0, h - 1, H)
        if main:
            for t in sorted({x[1] // 4 for x in order if x[2]} - {0}):
                prep(h, t)
        zc = [0]

        def zero():
            zc[0] += 1
            return z_s[zc[0] - 1]
        never = zv_s[zero()] != 0
        o = [jnp.zeros((DH, TQ), f32) for _ in range(NB)] + [o_prev]
        l = [[None] * 4 for _ in range(NB)]
        vcnt = {}

        def addl(b, j, v):
            l[b][j] = v if l[b][j] is None else l[b][j] + v

        def do_qk(i):
            b, ci, r0 = order[i]
            z = zero()
            kc = pltpu.bitcast(k_s[g + z, pl.ds((ci * KC + r0) // 2, (KC - r0) // 2), :], bf16)
            qm = pltpu.bitcast(qm_s[z, :, pl.ds(b * TQ, TQ)], bf16)
            p = jnp.exp2(jnp.dot(kc, qm, preferred_element_type=f32))
            for r in range((KC - r0) // 8):
                for j in range(4):
                    addl(b, j, p[8 * r:8 * r + 8, 128 * j:128 * j + 128])
                    for pb, c, a in attach.get((i, r, j), []):
                        ps = do_vpu(pb, c, a, j)
                        if pb != b:
                            lacc[pb][0, 1 + c * 2 + a, :, pl.ds(j * 128, 128)] = ps
                            l[b][j] = jnp.where(never, ps, l[b][j])
                        else:
                            addl(b, j, ps)
            bufof[(b, ci)][0, pl.ds(r0 // 2, (KC - r0) // 2), :] = _pack_rows(p)
            if i == no - 1 or order[i + 1][0] != b:
                lacc[b][0, 0] = jnp.concatenate(l[b], axis=-1)

        def do_vpu(b, c, a, j):
            t, sb = divmod(c, 4)
            acc = None
            z = zero()
            hq = h + z
            for d in range(DH):
                kbd = kbs[t][z, d, pl.ds(sb * 32 + a * 16, 16), :]
                qd = qf_s[hq, pl.ds(d, 1), pl.ds(b * TQ + j * 128, 128)]
                tt = kbd * qd
                acc = tt if acc is None else acc + tt
            p = jnp.exp2(acc)
            bufof[(b, c)][0, pl.ds(a * 8, 8), pl.ds(j * 128, 128)] = _pack_rows(p)
            vcnt[(b, c)] = vcnt.get((b, c), 0) + 4
            return p[0:8] + p[8:16]
        done = [0] * NB + [NC - LAG]

        def do_pv(i):
            prev = i < 0
            b, ci, r0 = order[i % no]
            assert prev or vcnt.get((b, ci), 0) == r0
            ob = NB if prev else b
            z = zero()
            h8 = pl.multiple_of((hp if prev else h) * 8, 8)
            vt = pltpu.bitcast(vt_s[pl.ds(h8, 8), pl.ds(ci * KC, KC)], bf16)
            o[ob] = o[ob] + jnp.dot(vt, pltpu.bitcast(bufof[(b, ci)][z], bf16), preferred_element_type=f32)
            done[ob] += 1
            if done[ob] == NC:
                cols = []
                for j in range(4):
                    v = lacc[b][z, 0, :, pl.ds(j * 128, 128)]
                    for sub in foreign[(b, j)]:
                        v = v + lacc[b][z, 1 + sub, :, pl.ds(j * 128, 128)]
                    cols.append(v)
                lsum = jnp.sum(jnp.concatenate(cols, axis=-1), axis=0, keepdims=True)
                hoff = pl.multiple_of((hpo if prev else h) * DH, DH)
                ot_s[pl.ds(hoff, DH), pl.ds(b * TQ, TQ)] = o[ob] * (1.0 / lsum)
        for i in range(no if main else LAG):
            if main:
                do_qk(i)
            do_pv(i - LAG)
        assert zc[0] <= NZ
        if main:
            set_q((h + 1) % H)
            if NPF:
                prep((h + 1) % H, 0)
            return o[NB - 1]

    def head_safe(h, c):
        g = h // 8
        hoff = pl.multiple_of(h * DH, DH)
        h8 = pl.multiple_of(h * 8, 8)
        set_q(h)

        def blk(b, c2):
            q0 = pl.multiple_of(b * TQ, TQ)
            qm = pltpu.bitcast(qm_s[0, :, pl.ds(q0, TQ)], bf16)
            m = jnp.full((8, TQ), -jnp.inf, f32)
            for c0 in range(0, S, 256):
                kc = pltpu.bitcast(k_s[g, pl.ds(c0 // 2, 128), :], bf16)
                s = jnp.dot(kc, qm, preferred_element_type=f32)
                sc_s[pl.ds(c0, 256), :] = s
                m = jnp.maximum(m, jnp.max(s.reshape(32, 8, TQ), axis=0))
            m = jnp.max(m, axis=0, keepdims=True)
            l = jnp.zeros((8, TQ), f32)
            o = jnp.zeros((DH, TQ), f32)
            for c0 in range(0, S, 256):
                p = jnp.exp2(sc_s[pl.ds(c0, 256), :] - m)
                l = l + jnp.sum(p.reshape(32, 8, TQ), axis=0)
                vt = pltpu.bitcast(vt_s[pl.ds(h8, 8), pl.ds(c0, 256)], bf16)
                o = o + jnp.dot(vt, pltpu.bitcast(_pack_rows(p), bf16), preferred_element_type=f32)
            ot_s[pl.ds(hoff, DH), pl.ds(q0, TQ)] = o * (1.0 / jnp.sum(l, axis=0, keepdims=True))
            return c2
        lax.fori_loop(0, NB, blk, 0)
        return c

    def attention():
        qn = jnp.max(st_s[0], axis=1, keepdims=True)
        kn = jnp.max(st_s[1], axis=1, keepdims=True)
        bound2 = jnp.max(qn * kn) * 1.05
        vmax = jnp.max(st_s[2])
        st_s[...] = jnp.zeros_like(st_s)
        ok = jnp.logical_and(bound2 <= SAFE_LOG2 * SAFE_LOG2,
                             jnp.logical_and(vmax <= 2.0 ** 40, vmax >= 2.0 ** -30))

        @pl.when(ok)
        def _():
            set_q(0)
            o_last = lax.fori_loop(0, H, head_fast, jnp.zeros((DH, TQ), f32))
            head_fast(H, o_last, main=False)

        @pl.when(jnp.logical_not(ok))
        def _():
            lax.fori_loop(0, H, head_safe, 0)

    def dense(last):
        def body(r, c):
            r0s = [pl.multiple_of(r * TI + t * TR, TR) for t in range(NT)]
            if not last:
                prep(0, 0)
            xs = []
            for r0 in r0s:
                o = ot_s[pl.ds(0, D), pl.ds(r0, TR)].T.astype(bf16)
                xs.append(xres[pl.ds(r0, TR), :] + jnp.dot(o, wo_ref[...], preferred_element_type=f32))
            hs = []
            for x in xs:
                xn = _ln(x).astype(bf16)
                hh = jnp.dot(xn, w1_ref[...], preferred_element_type=f32) + b1_ref[...].astype(f32)
                hs.append(_gelu(hh).astype(bf16))
            xs = [x + jnp.dot(hh, w2_ref[...], preferred_element_type=f32) + b2_ref[...].astype(f32)
                  for x, hh in zip(xs, hs)]
            kh = []
            for r0, x in zip(r0s, xs):
                if last:
                    x_ref[pl.ds(r0, TR), :] = x.astype(bf16)
                else:
                    xres[pl.ds(r0, TR), :] = x
                    kh += proj(r0, x)
            if last:
                o_copy(r).start()
            else:
                put_kt(r, kh)
            return c
        lax.fori_loop(0, S // TI, body, 0)

    def layer(i, c):
        attention()

        @pl.when(i == 0)
        def _():
            for cp in w_copies[1:]:
                cp.wait()
            dense(False)

        @pl.when(i == 1)
        def _():
            dense(True)
        return c
    lax.fori_loop(0, 2, layer, 0)
    for r in range(S // TI):
        o_copy(r).wait()


@jax.jit
def pallas_interleave_layers__mha_block__dense_activation_gelu__prompt_kernel(A_x, A_wqkv, A_wo, B_x, B_w1, B_b1, B_w2, B_b2):
    x = A_x.reshape(S, D)
    hbm = pl.BlockSpec(memory_space=pl.ANY)
    vmem = pl.BlockSpec(memory_space=pltpu.VMEM)
    out = pl.pallas_call(
        _kernel,
        out_shape=jax.ShapeDtypeStruct((S, D), bf16),
        in_specs=[hbm, hbm, hbm, hbm, vmem, hbm, vmem],
        out_specs=hbm,
        scratch_shapes=[
            pltpu.VMEM((S, D), bf16),
            pltpu.VMEM((D, 3 * D), bf16),
            pltpu.VMEM((D, D), bf16),
            pltpu.VMEM((D, F), bf16),
            pltpu.VMEM((F, D), bf16),
            pltpu.SemaphoreType.DMA((S // TI,)),
            pltpu.SemaphoreType.DMA((4,)),
            pltpu.SemaphoreType.DMA((S // TI,)),
            pltpu.VMEM((S, D), f32),
            pltpu.VMEM((D, D), bf16),
            pltpu.VMEM((D, D), bf16),
            pltpu.VMEM((4, S // 2, 128), u32),
            pltpu.VMEM((D // 2, S), u32),
            pltpu.VMEM((D // 2, S), u32),
            pltpu.VMEM((H, DH, S), f32),
            pltpu.VMEM((4, H, DH, 128), f32),
            pltpu.VMEM((D + DH, S), f32),
            pltpu.VMEM((1, 64, S), u32),
            pltpu.VMEM((3, H, TR), f32),
            pltpu.VMEM((S, TQ), f32),
            pltpu.VMEM((4, 8, 128), jnp.int32),
            pltpu.SMEM((NZ,), jnp.int32),
        ] + [pltpu.VMEM((1, 64, TQ), u32) for _ in range(NR)]
          + [pltpu.VMEM((1, DH, 128, 128), f32) for _ in range(NVM)]
          + [pltpu.VMEM((1, NL, 8, TQ), f32) for _ in range(NB)],
        compiler_params=pltpu.CompilerParams(vmem_limit_bytes=100 * 2 ** 20),
    )(x, A_wqkv, A_wo, B_w1, B_b1.reshape(1, F), B_w2, B_b2.reshape(1, D))
    return out.reshape(1, S, D)
```

```python
import jax
import jax.numpy as jnp
from jax import lax
import jax.experimental.pallas as pl
import jax.experimental.pallas.tpu as pltpu

S, D, H, DH, F = 2048, 512, 32, 16, 1792
TR = 128
NT = 4
TI = TR * NT
TQ = 512
KC = 128
NB = S // TQ
NC = S // KC
LAG = 4
NS = (5, 9, 9, 9)
START = 16
PVM = 2
NPF = 3


def _groups(first, n):
    out = [(first + i, 32) for i in range(int(n))]
    if n != int(n):
        out.append((first + int(n), 16))
    return out


SUBS = [_groups(4, n) for n in NS]
SUBS[0] = _groups(0, NPF) + SUBS[0]
NVM = 4
NR = 16
NL = 36
NZ = 600
LOG2E = 1.4426950408889634
QSCALE = (DH ** -0.5) * LOG2E
SAFE_LOG2 = 60.0
bf16 = jnp.bfloat16
f32 = jnp.float32
u32 = jnp.uint32


def _ln(x):
    m = jnp.mean(x, axis=-1, keepdims=True)
    xc = x - m
    v = jnp.mean(xc * xc, axis=-1, keepdims=True)
    return xc * lax.rsqrt(v + 1e-5)


def _gelu(x):
    c = 0.7978845608028654
    return 0.5 * x * (1.0 + jnp.tanh(c * (x + 0.044715 * (x * x * x))))


def _plan():
    nrows = sum(NC * 16 - sum(r // 8 for _, r in x) for x in SUBS)
    pieces = [(b, c, a, j) for b in range(NB) for c, r in SUBS[b] for a in range(r // 16) for j in range(4)]
    pos = {pc: START + int((k + 0.5) * (nrows - START) / len(pieces)) for k, pc in enumerate(pieces)}
    order = []
    row = 0
    for b in range(NB):
        mixed = list(SUBS[b])
        pure = [c for c in range(NC) if c not in dict(mixed)]
        while mixed or pure:
            if mixed and (not pure or row + (LAG - PVM) * 14 > pos[(b, mixed[0][0], mixed[0][1] // 16 - 1, 3)]):
                order.append((b,) + mixed.pop(0))
            else:
                order.append((b, pure.pop(0), 0))
            row += 16 - order[-1][2] // 8
    rows = [(i, r) for i, x in enumerate(order) for r in range(16 - x[2] // 8)]
    attach = {}
    foreign = {(b, j): [] for b in range(NB) for j in range(4)}
    for (pb, c, a, j), p in pos.items():
        i, r = rows[p]
        attach.setdefault((i, r, j), []).append((pb, c, a))
        if pb != order[i][0]:
            foreign[(pb, j)].append(c * 2 + a)
    return order, attach, foreign


def _kernel(x_hbm, wqkv_hbm, wo_hbm, w1_hbm, b1_ref, w2_hbm, b2_ref, o_hbm,
            x_ref, wqkv_ref, wo_ref, w1_ref, w2_ref, sem_x, sem_w, sem_o,
            xres, wqt, wvt, k_s, qt_s, vt_s, qf_s, kt_s, ot_s, qm_s, st_s, sc_s, zv_s, z_s, *bufs):
    ring = bufs[:NR]
    kbs = bufs[NR:NR + NVM]
    lacc = bufs[NR + NVM:]

    def x_copy(r):
        rows = pl.ds(pl.multiple_of(r * TI, TI), TI)
        return pltpu.make_async_copy(x_hbm.at[rows], x_ref.at[rows], sem_x.at[r])

    def o_copy(r):
        rows = pl.ds(pl.multiple_of(r * TI, TI), TI)
        return pltpu.make_async_copy(x_ref.at[rows], o_hbm.at[rows], sem_o.at[r])
    w_copies = [pltpu.make_async_copy(a, b, sem_w.at[i]) for i, (a, b) in enumerate(
        [(wo_hbm, wo_ref), (w1_hbm, w1_ref), (w2_hbm, w2_ref)])]
    qkv_copies = [pltpu.make_async_copy(wqkv_hbm.at[:, pl.ds(i * D, D)], wqkv_ref.at[i], sem_w.at[3 + i])
                  for i in range(3)]
    qkv_copies[0].start()
    qkv_copies[2].start()
    x_copy(0).start()
    qkv_copies[1].start()
    qm_s[...] = jnp.zeros_like(qm_s)
    st_s[...] = jnp.zeros_like(st_s)
    zv_s[...] = jnp.zeros_like(zv_s)
    kt_s[0, 0] = jnp.zeros((DH, 128), f32)
    for buf in ring[NR - LAG:]:
        buf[...] = jnp.zeros_like(buf)
    lacc[NB - 1][...] = jnp.ones_like(lacc[NB - 1])
    for i in range(NZ):
        z_s[i] = 0
    qkv_copies[0].wait()
    for r in range(1, S // TI):
        x_copy(r).start()
    wqt[...] = wqkv_ref[0].astype(f32).T.astype(bf16)
    qkv_copies[2].wait()
    wvt[...] = wqkv_ref[2].astype(f32).T.astype(bf16)
    qkv_copies[1].wait()

    nt = (((1,), (1,)), ((), ()))

    def proj(r0, x):
        xn = _ln(x)
        xb = xn.astype(bf16)
        k = jnp.dot(xb, wqkv_ref[1], preferred_element_type=f32)
        kp = pltpu.bitcast(k.astype(bf16), u32)
        r2 = pl.multiple_of(r0 // 2, TR // 2)
        for g in range(4):
            k_s[g, pl.ds(r2, TR // 2), :] = kp[:, g * 128:(g + 1) * 128]
        kt = k.T.reshape(H, DH, TR)
        q = lax.dot_general(wqt[...], xb, nt, preferred_element_type=f32) * QSCALE
        qt_s[:, pl.ds(r0, TR)] = pltpu.bitcast(q.astype(bf16), u32)
        q3 = q.reshape(H, DH, TR)
        qf_s[:, :, pl.ds(r0, TR)] = q3
        v = lax.dot_general(wvt[...], xb, nt, preferred_element_type=f32)
        vt_s[:, pl.ds(r0, TR)] = pltpu.bitcast(v.astype(bf16), u32)
        st_s[0] = jnp.maximum(st_s[0], jnp.sum(q3 * q3, axis=1))
        st_s[1] = jnp.maximum(st_s[1], jnp.sum(kt * kt, axis=1))
        st_s[2] = jnp.maximum(st_s[2], jnp.max(jnp.abs(v).reshape(DH, H, TR), axis=0))

        return [k[c0:c0 + 32] for c0 in range(0, TR, KC)]

    def prep(h, t):
        for d in range(DH):
            row = jnp.broadcast_to(kt_s[t, h, pl.ds(d, 1), :], (128, 128))
            kbs[t][0, d] = row.T

    def put_kt(r, heads):
        kt_s[r] = jnp.concatenate(heads, axis=0).T.reshape(H, DH, 128)

    def first(r, c):
        x_copy(r).wait()
        prep(0, 0)
        kh = []
        for t in range(NT):
            r0 = pl.multiple_of(r * TI + t * TR, TR)
            x = x_ref[pl.ds(r0, TR), :].astype(f32)
            xres[pl.ds(r0, TR), :] = x
            kh += proj(r0, x)
        put_kt(r, kh)
        return c
    lax.fori_loop(0, S // TI, first, 0)
    for cp in w_copies:
        cp.start()

    def set_q(h):
        moff = pl.multiple_of((h % 8) * 8, 8)
        poff = pl.multiple_of(((h + 7) % 8) * 8, 8)
        qm_s[0, pl.ds(poff, 8), :] = jnp.zeros((8, S), u32)
        qm_s[0, pl.ds(moff, 8), :] = qt_s[pl.ds(pl.multiple_of(h * 8, 8), 8), :]

    order, attach, foreign = _plan()
    no = len(order)
    bufof = {x[:2]: ring[i % NR] for i, x in enumerate(order)}

    def head_fast(h, o_prev, main=True):
        g = h // 8
        hp = jnp.maximum(h - 1, 0)
        hpo = jnp.where(h > 0, h - 1, H)
        if main:
            for t in sorted({x[1] // 4 for x in order if x[2]} - {0}):
                prep(h, t)
        zc = [0]

        def zero():
            zc[0] += 1
            return z_s[zc[0] - 1]
        never = zv_s[zero()] != 0
        o = [jnp.zeros((DH, TQ), f32) for _ in range(NB)] + [o_prev]
        l = [[None] * 4 for _ in range(NB)]
        vcnt = {}

        def addl(b, j, v):
            l[b][j] = v if l[b][j] is None else l[b][j] + v

        def do_qk(i):
            b, ci, r0 = order[i]
            z = zero()
            kc = pltpu.bitcast(k_s[g + z, pl.ds((ci * KC + r0) // 2, (KC - r0) // 2), :], bf16)
            qm = pltpu.bitcast(qm_s[z, :, pl.ds(b * TQ, TQ)], bf16)
            p = jnp.exp2(jnp.dot(kc, qm, preferred_element_type=f32))
            nr = (KC - r0) // 8
            p3 = p.reshape(nr, 8, TQ)
            nxt = [0] * 4

            def flush(j, upto):
                if upto > nxt[j]:
                    seg = p3[nxt[j]:upto, :, 128 * j:128 * j + 128]
                    if l[b][j] is not None:
                        seg = jnp.concatenate([l[b][j][None], seg], axis=0)
                    l[b][j] = jnp.sum(seg, axis=0)
                    nxt[j] = upto
            for r in range(nr):
                for j in range(4):
                    for pb, c, a in attach.get((i, r, j), []):
                        flush(j, r + 1)
                        ps = do_vpu(pb, c, a, j)
                        if pb != b:
                            lacc[pb][0, 1 + c * 2 + a, :, pl.ds(j * 128, 128)] = ps
                            l[b][j] = jnp.where(never, ps, l[b][j])
                        else:
                            addl(b, j, ps)
            for j in range(4):
                flush(j, nr)
            for j in range(4):
                bufof[(b, ci)][0, j, pl.ds(r0, KC - r0), :] = p[:, 128 * j:128 * j + 128].astype(bf16)
            if i == no - 1 or order[i + 1][0] != b:
                lacc[b][0, 0] = jnp.concatenate(l[b], axis=-1)

        def do_vpu(b, c, a, j):
            t, sb = divmod(c, 4)
            acc = None
            z = zero()
            hq = h + z
            for d in range(DH):
                kbd = kbs[t][z, d, pl.ds(sb * 32 + a * 16, 16), :]
                qd = qf_s[hq, pl.ds(d, 1), pl.ds(b * TQ + j * 128, 128)]
                tt = kbd * qd
                acc = tt if acc is None else acc + tt
            p = jnp.exp2(acc)
            bufof[(b, c)][0, j, pl.ds(a * 16, 16), :] = p.astype(bf16)
            vcnt[(b, c)] = vcnt.get((b, c), 0) + 4
            return p[0:8] + p[8:16]
        done = [0] * NB + [NC - LAG]

        def do_pv(i):
            prev = i < 0
            b, ci, r0 = order[i % no]
            assert prev or vcnt.get((b, ci), 0) == r0
            ob = NB if prev else b
            z = zero()
            h8 = pl.multiple_of((hp if prev else h) * 8, 8)
            vt = pltpu.bitcast(vt_s[pl.ds(h8, 8), pl.ds(ci * KC, KC)], bf16)
            o[ob] = o[ob] + jnp.dot(vt, jnp.concatenate([pltpu.bitcast(bufof[(b, ci)].bitcast(u32)[z, j], bf16) for j in range(4)], axis=1), preferred_element_type=f32)
            done[ob] += 1
            if done[ob] == NC:
                cols = []
                for j in range(4):
                    v = lacc[b][z, 0, :, pl.ds(j * 128, 128)]
                    for sub in foreign[(b, j)]:
                        v = v + lacc[b][z, 1 + sub, :, pl.ds(j * 128, 128)]
                    cols.append(v)
                lsum = jnp.sum(jnp.concatenate(cols, axis=-1), axis=0, keepdims=True)
                hoff = pl.multiple_of((hpo if prev else h) * DH, DH)
                ot_s[pl.ds(hoff, DH), pl.ds(b * TQ, TQ)] = o[ob] * (1.0 / lsum)
        for i in range(no if main else LAG):
            if main:
                do_qk(i)
            do_pv(i - LAG)
        assert zc[0] <= NZ
        if main:
            set_q((h + 1) % H)
            if NPF:
                prep((h + 1) % H, 0)
            return o[NB - 1]

    def head_safe(h, c):
        g = h // 8
        hoff = pl.multiple_of(h * DH, DH)
        h8 = pl.multiple_of(h * 8, 8)
        set_q(h)

        def blk(b, c2):
            q0 = pl.multiple_of(b * TQ, TQ)
            qm = pltpu.bitcast(qm_s[0, :, pl.ds(q0, TQ)], bf16)
            m = jnp.full((8, TQ), -jnp.inf, f32)
            for c0 in range(0, S, 256):
                kc = pltpu.bitcast(k_s[g, pl.ds(c0 // 2, 128), :], bf16)
                s = jnp.dot(kc, qm, preferred_element_type=f32)
                sc_s[pl.ds(c0, 256), :] = s
                m = jnp.maximum(m, jnp.max(s.reshape(32, 8, TQ), axis=0))
            m = jnp.max(m, axis=0, keepdims=True)
            l = jnp.zeros((8, TQ), f32)
            o = jnp.zeros((DH, TQ), f32)
            for c0 in range(0, S, 256):
                p = jnp.exp2(sc_s[pl.ds(c0, 256), :] - m)
                l = l + jnp.sum(p.reshape(32, 8, TQ), axis=0)
                vt = pltpu.bitcast(vt_s[pl.ds(h8, 8), pl.ds(c0, 256)], bf16)
                o = o + jnp.dot(vt, p.astype(bf16), preferred_element_type=f32)
            ot_s[pl.ds(hoff, DH), pl.ds(q0, TQ)] = o * (1.0 / jnp.sum(l, axis=0, keepdims=True))
            return c2
        lax.fori_loop(0, NB, blk, 0)
        return c

    def attention():
        qn = jnp.max(st_s[0], axis=1, keepdims=True)
        kn = jnp.max(st_s[1], axis=1, keepdims=True)
        bound2 = jnp.max(qn * kn) * 1.05
        vmax = jnp.max(st_s[2])
        st_s[...] = jnp.zeros_like(st_s)
        ok = jnp.logical_and(bound2 <= SAFE_LOG2 * SAFE_LOG2,
                             jnp.logical_and(vmax <= 2.0 ** 40, vmax >= 2.0 ** -30))

        @pl.when(ok)
        def _():
            set_q(0)
            o_last = lax.fori_loop(0, H, head_fast, jnp.zeros((DH, TQ), f32))
            head_fast(H, o_last, main=False)

        @pl.when(jnp.logical_not(ok))
        def _():
            lax.fori_loop(0, H, head_safe, 0)

    def dense(last):
        def body(r, c):
            r0s = [pl.multiple_of(r * TI + t * TR, TR) for t in range(NT)]
            if not last:
                prep(0, 0)
            xs = []
            for r0 in r0s:
                o = ot_s[pl.ds(0, D), pl.ds(r0, TR)].T.astype(bf16)
                xs.append(xres[pl.ds(r0, TR), :] + jnp.dot(o, wo_ref[...], preferred_element_type=f32))
            hs = []
            for x in xs:
                xn = _ln(x).astype(bf16)
                hh = jnp.dot(xn, w1_ref[...], preferred_element_type=f32) + b1_ref[...].astype(f32)
                hs.append(_gelu(hh).astype(bf16))
            xs = [x + jnp.dot(hh, w2_ref[...], preferred_element_type=f32) + b2_ref[...].astype(f32)
                  for x, hh in zip(xs, hs)]
            kh = []
            for r0, x in zip(r0s, xs):
                if last:
                    x_ref[pl.ds(r0, TR), :] = x.astype(bf16)
                else:
                    xres[pl.ds(r0, TR), :] = x
                    kh += proj(r0, x)
            if last:
                o_copy(r).start()
            else:
                put_kt(r, kh)
            return c
        lax.fori_loop(0, S // TI, body, 0)

    def layer(i, c):
        attention()

        @pl.when(i == 0)
        def _():
            for cp in w_copies:
                cp.wait()
            dense(False)

        @pl.when(i == 1)
        def _():
            dense(True)
        return c
    lax.fori_loop(0, 2, layer, 0)
    for r in range(S // TI):
        o_copy(r).wait()


@jax.jit
def pallas_interleave_layers__mha_block__dense_activation_gelu__prompt_kernel(A_x, A_wqkv, A_wo, B_x, B_w1, B_b1, B_w2, B_b2):
    x = A_x.reshape(S, D)
    hbm = pl.BlockSpec(memory_space=pl.ANY)
    vmem = pl.BlockSpec(memory_space=pltpu.VMEM)
    out = pl.pallas_call(
        _kernel,
        out_shape=jax.ShapeDtypeStruct((S, D), bf16),
        in_specs=[hbm, hbm, hbm, hbm, vmem, hbm, vmem],
        out_specs=hbm,
        scratch_shapes=[
            pltpu.VMEM((S, D), bf16),
            pltpu.VMEM((3, D, D), bf16),
            pltpu.VMEM((D, D), bf16),
            pltpu.VMEM((D, F), bf16),
            pltpu.VMEM((F, D), bf16),
            pltpu.SemaphoreType.DMA((S // TI,)),
            pltpu.SemaphoreType.DMA((6,)),
            pltpu.SemaphoreType.DMA((S // TI,)),
            pltpu.VMEM((S, D), f32),
            pltpu.VMEM((D, D), bf16),
            pltpu.VMEM((D, D), bf16),
            pltpu.VMEM((4, S // 2, 128), u32),
            pltpu.VMEM((D // 2, S), u32),
            pltpu.VMEM((D // 2, S), u32),
            pltpu.VMEM((H, DH, S), f32),
            pltpu.VMEM((4, H, DH, 128), f32),
            pltpu.VMEM((D + DH, S), f32),
            pltpu.VMEM((1, 64, S), u32),
            pltpu.VMEM((3, H, TR), f32),
            pltpu.VMEM((S, TQ), f32),
            pltpu.VMEM((4, 8, 128), jnp.int32),
            pltpu.SMEM((NZ,), jnp.int32),
        ] + [pltpu.VMEM((1, 4, KC, 128), bf16) for _ in range(NR)]
          + [pltpu.VMEM((1, DH, 128, 128), f32) for _ in range(NVM)]
          + [pltpu.VMEM((1, NL, 8, TQ), f32) for _ in range(NB)],
        compiler_params=pltpu.CompilerParams(vmem_limit_bytes=100 * 2 ** 20),
    )(x, A_wqkv, A_wo, B_w1, B_b1.reshape(1, F), B_w2, B_b2.reshape(1, D))
    return out.reshape(1, S, D)
```

```python
import jax
import jax.numpy as jnp
from jax import lax
import jax.experimental.pallas as pl
import jax.experimental.pallas.tpu as pltpu

S, D, H, DH, F = 2048, 512, 32, 16, 1792
TR = 128
NT1 = 4
NT2 = 4
NT3 = 4
TI = 512
TO = 128
TQ = 512
KC = 128
NB = S // TQ
NC = S // KC
LAG = 4
NS = (4.5, 9, 10.5, 9)
START = 4
PVM = 2
NPF = 3


def _groups(first, n):
    out = [(first + i, 32) for i in range(int(n))]
    if n != int(n):
        out.append((first + int(n), 16))
    return out


NP0 = (3, 0, 0, 0)
SUBS = [_groups(0, m) + _groups(4, n) for m, n in zip(NP0, NS)]
NVM = 4
NR = 16
RG = 256
CWK = 128
GS = 80
SF1 = 1
SF2 = 1
SWO = 0
SK = 1
SQ = 1
FH = 896
CW = 256
CW1 = 128
KPAD = 24
RPAD = 16
QPAD = 0
W1 = 0.9
Z1 = 170
W2 = 0.95
Z2 = 90
ORD = 0
RPS = 14
NCH = 2
QF = 0
NL = 36
NZ = 600
LOG2E = 1.4426950408889634
QSCALE = (DH ** -0.5) * LOG2E
SAFE_LOG2 = 60.0
bf16 = jnp.bfloat16
f32 = jnp.float32
u32 = jnp.uint32


def _ln(x):
    m = jnp.mean(x, axis=-1, keepdims=True)
    xc = x - m
    v = jnp.mean(xc * xc, axis=-1, keepdims=True)
    return xc * lax.rsqrt(v + 1e-5)


def _gelu(x):
    c = 0.7978845608028654
    return 0.5 * x * (1.0 + jnp.tanh(c * (x + 0.044715 * (x * x * x))))


def _lhs_combos(a1, a2, kh):
    a11, a12, a21, a22 = a1[:, :kh], a1[:, kh:2 * kh], a2[:, :kh], a2[:, kh:2 * kh]
    return [t.astype(bf16) for t in (a11 + a22, a21 + a22, a11, a22, a11 + a12, a21 - a11, a12 - a22)]


def _rhs_combos(w_ref, c_ref, kh, part, transposed=False, row0=0):
    nh = c_ref.shape[2]
    units = kh // 16
    per = -(-units // 3)
    start = jnp.minimum(part * per, units - per)

    def job(u, c0, w):
        def run():
            r = pl.multiple_of((start + u) * 16, 16)
            b11, b12, b21, b22 = (w_ref[pl.ds(rr, 16), pl.ds(cc, w)].astype(f32)
                                  for rr in (r, kh + r) for cc in (c0, nh + c0))
            if transposed:
                b12, b21 = b21, b12
            r2 = pl.multiple_of(row0 + (start + u) * 8, 8)
            tok = None
            for n, t in enumerate((b11 + b22, b11, b12 - b22, b21 - b11, b22, b11 + b12, b21 + b22)):
                t = pltpu.bitcast(t.astype(bf16), u32)
                c_ref[n, pl.ds(r2, 8), pl.ds(c0, w)] = t
                for l0 in range(0, w, 128):
                    tok = t[:, l0:l0 + 128] if tok is None else tok | t[:, l0:l0 + 128]
            return pltpu.bitcast(tok, f32)
        return run
    return [job(u, c0, min(256, nh - c0)) for u in range(per) for c0 in range(0, nh, 256)]


def _strassen(ac, c_ref, cw, z):
    nh = c_ref.shape[2]
    out = [[], [], [], []]
    for c0 in range(0, nh, cw):
        w = min(cw, nh - c0)

        def m(i):
            return jnp.dot(ac[i], pltpu.bitcast(c_ref[i + z, :, c0:c0 + w], bf16), preferred_element_type=f32)
        m2, m4 = m(1), m(3)
        out[2].append(m2 + m4)
        m1 = m(0)
        t11, t22 = m1 + m4, m1 - m2
        m3 = m(2)
        t22 = t22 + m3
        m5 = m(4)
        out[1].append(m3 + m5)
        out[0].append(t11 - m5 + m(6))
        out[3].append(t22 + m(5))
    return [jnp.concatenate(o, axis=1) if len(o) > 1 else o[0] for o in out]


def _strassen_t(ac, c_ref, z):
    out = [[], [], [], []]
    for r0 in range(0, c_ref.shape[1], RG // 2):
        def m(i):
            return lax.dot_general(pltpu.bitcast(c_ref[i + z, r0:r0 + RG // 2, :], bf16), ac[i],
                                   (((1,), (1,)), ((), ())), preferred_element_type=f32)
        m2, m4 = m(1), m(3)
        out[2].append(m2 + m4)
        m1, m3 = m(0), m(2)
        t11, t22 = m1 + m4, m1 - m2 + m3
        m5 = m(4)
        out[1].append(m3 + m5)
        out[0].append(t11 - m5 + m(6))
        out[3].append(t22 + m(5))
    return [jnp.concatenate(o, axis=0) if len(o) > 1 else o[0] for o in out]


def _plan():
    nrows = sum(NC * 16 - sum(r // 8 for _, r in x) for x in SUBS)
    if ORD:
        pieces = [(b, c, a, j) for b in range(NB) for c, r in SUBS[b] for j in range(4) for a in range(r // 16)]
    else:
        pieces = [(b, c, a, j) for b in range(NB) for c, r in SUBS[b] for a in range(r // 16) for j in range(4)]
    wts = [0.0 if r < START else W1 if r < Z1 else W2 if r >= nrows - Z2 else 1.0 for r in range(nrows)]
    pos = {}
    row, cum = 0, 0.0
    for k, pc in enumerate(pieces):
        while cum + wts[row] <= (k + 0.5) * sum(wts) / len(pieces):
            cum += wts[row]
            row += 1
        pos[pc] = row
    order = []
    row = 0
    for b in range(NB):
        mixed = list(SUBS[b])
        pure = [c for c in range(NC) if c not in dict(mixed)]
        while mixed or pure:
            if mixed and (not pure or row + (LAG - PVM) * RPS > pos[(b, mixed[0][0], mixed[0][1] // 16 - 1, 3)]):
                order.append((b,) + mixed.pop(0))
            else:
                order.append((b, pure.pop(0), 0))
            row += 16 - order[-1][2] // 8
    rows = [(i, r) for i, x in enumerate(order) for r in range(16 - x[2] // 8)]
    attach = {}
    foreign = {(b, j): [] for b in range(NB) for j in range(4)}
    for (pb, c, a, j), p in pos.items():
        i, r = rows[p]
        attach.setdefault((i, r, j), []).append((pb, c, a))
        if pb != order[i][0]:
            foreign[(pb, j)].append(c * 2 + a)
    return order, attach, foreign


def _kernel(x_hbm, wqkv_hbm, wo_hbm, w1_hbm, b1_hbm, w2_hbm, b2_hbm, o_hbm,
            x_ref, wqkv_ref, wo_ref, w1_ref, w2_ref, sem_x, sem_w, sem_o,
            xres, wqt, wvt, k_s, qt_s, vt_s, qf_s, kt_s, ot_s, qm_s, st_s, sc_s, zv_s, bias_s, z_s, *bufs):
    ring = bufs[:NR]
    kbs = bufs[NR:NR + NVM]
    lacc = bufs[NR + NVM:NR + NVM + NB]
    b1_ref, b2_ref, w1c, w2c, woc, wkc, wqvc = bufs[NR + NVM + NB:]

    def x_copy(r):
        rows = pl.ds(pl.multiple_of(r * TI, TI), TI)
        return pltpu.make_async_copy(x_hbm.at[rows], x_ref.at[rows], sem_x.at[r])

    def o_copy(r):
        rows = pl.ds(pl.multiple_of(r * TO, TO), TO)
        return pltpu.make_async_copy(x_ref.at[rows], o_hbm.at[rows], sem_o.at[r])
    w_copies = [pltpu.make_async_copy(a, b, sem_w.at[i]) for i, (a, b) in enumerate(
        [(wo_hbm, wo_ref), (b1_hbm, b1_ref.at[pl.ds(0, F)]), (b2_hbm, b2_ref.at[pl.ds(0, D)])])]
    qkv_copies = [pltpu.make_async_copy(wqkv_hbm.at[:, pl.ds(i * D, D)], wqkv_ref.at[i], sem_w.at[3 + i])
                  for i in range(3)]
    ffn_copies = [[], []]
    for src, dst in ((w1_hbm, w1_ref), (w2_hbm, w2_ref)):
        kh = src.shape[0] // 2
        cut = -(-(kh // 16) // 3) * 16
        for half in (0, kh):
            for stage, rows in enumerate((pl.ds(half, cut), pl.ds(half + cut, kh - cut))):
                sem = sem_w.at[6 + len(ffn_copies[0]) + len(ffn_copies[1])]
                ffn_copies[stage].append(pltpu.make_async_copy(src.at[rows], dst.at[rows], sem))
    x_copy(0).start()
    qkv_copies[1].start()
    qkv_copies[0].start()
    qkv_copies[2].start()
    qm_s[...] = jnp.zeros_like(qm_s)
    st_s[...] = jnp.zeros_like(st_s)
    zv_s[...] = jnp.zeros_like(zv_s)
    for buf in ring[NR - LAG:]:
        buf[...] = jnp.zeros_like(buf)
    lacc[NB - 1][...] = jnp.ones_like(lacc[NB - 1])
    for i in range(NZ):
        z_s[i] = 0

    nt = (((1,), (1,)), ((), ()))

    def put_k(r0, k):
        kp = pltpu.bitcast(k.astype(bf16), u32)
        r2 = pl.multiple_of(r0 // 2, TR // 2)
        for g in range(4):
            k_s[g, pl.ds(r2, TR // 2), :] = kp[:, g * 128:(g + 1) * 128]
        kt = k.T.reshape(H, DH, TR)
        st_s[1] = jnp.maximum(st_s[1], jnp.sum(kt * kt, axis=1))
        return [k[c0:c0 + 32] for c0 in range(0, TR, KC)]

    def put_qv(r0, q, v):
        q = q * QSCALE
        qt_s[:, pl.ds(r0, TR)] = pltpu.bitcast(q.astype(bf16), u32)
        q3 = q.reshape(H, DH, TR)
        qf_s[:, :, pl.ds(r0, TR)] = q3
        vt_s[:, pl.ds(r0, TR)] = pltpu.bitcast(v.astype(bf16), u32)
        st_s[0] = jnp.maximum(st_s[0], jnp.sum(q3 * q3, axis=1))
        st_s[2] = jnp.maximum(st_s[2], jnp.max(jnp.abs(v).reshape(DH, H, TR), axis=0))

    def proj_k(r0, xb):
        return put_k(r0, jnp.dot(xb, wqkv_ref[1], preferred_element_type=f32))

    def proj_qv(r0, xb, jobs=(), never=None):
        out = []
        for n, w in enumerate((wqt, wvt)):
            y = lax.dot_general(w[...], xb, nt, preferred_element_type=f32)
            mine = jobs[n::2]
            if mine:
                step = D // len(mine) // 8 * 8
                parts = []
                for i, run in enumerate(mine):
                    parts.append(jnp.where(never, run(), y[i * step:i * step + 8]))
                    parts.append(y[i * step + 8:(i + 1) * step if i + 1 < len(mine) else D])
                y = jnp.concatenate(parts, axis=0)
            out.append(y)
        put_qv(r0, *out)

    def proj2(r1, x1, r2, x2, z):
        n1, n2 = _ln(x1), _ln(x2)
        ac = _lhs_combos(n1, n2, D // 2)
        if SK:
            cs = _strassen(ac, wkc, CWK, z)
            kh = put_k(r1, jnp.concatenate(cs[:2], axis=1)) + put_k(r2, jnp.concatenate(cs[2:], axis=1))
        else:
            kh = proj_k(r1, n1.astype(bf16)) + proj_k(r2, n2.astype(bf16))
        if SQ:
            hd = D // 2
            cs = _strassen_t(ac, wqvc, z)
            put_qv(r1, jnp.concatenate([cs[0][:hd], cs[1][:hd]], axis=0), jnp.concatenate([cs[0][hd:], cs[1][hd:]], axis=0))
            put_qv(r2, jnp.concatenate([cs[2][:hd], cs[3][:hd]], axis=0), jnp.concatenate([cs[2][hd:], cs[3][hd:]], axis=0))
        else:
            proj_qv(r1, n1.astype(bf16))
            proj_qv(r2, n2.astype(bf16))
        return kh

    def prep(h, t):
        for d in range(DH):
            row = jnp.broadcast_to(kt_s[t, h, pl.ds(d, 1), :], (128, 128))
            kbs[t][0, d, pl.ds(0, 128), :] = row.T

    def put_kt(r, heads):
        for i in range(len(heads) // 4):
            kt_s[r * (len(heads) // 4) + i] = jnp.concatenate(heads[4 * i:4 * i + 4], axis=0).T.reshape(H, DH, 128)

    def first(r, c):
        kh = []

        @pl.when(r == 2)
        def _():
            for cp in ffn_copies[1]:
                cp.wait()
        x_copy(r).wait()
        prep(0, 0)
        never = zv_s[z_s[0]] != 0
        jobs = _rhs_combos(w1_ref, w1c, D // 2, r - 1) + _rhs_combos(w2_ref, w2c, FH, r - 1)
        if SK:
            jobs += _rhs_combos(wqkv_ref.at[1], wkc, D // 2, r - 1)
        if SQ:
            jobs += _rhs_combos(wqt, wqvc, D // 2, r - 1, True)
            jobs += _rhs_combos(wvt, wqvc, D // 2, r - 1, True, D // 4)
        for t in range(NT1):
            r0 = pl.multiple_of(r * (NT1 * TR) + t * TR, TR)
            x = x_ref[pl.ds(r0, TR), :].astype(f32)
            xres[pl.ds(r0, TR), :] = x
            xb = _ln(x).astype(bf16)
            kh += proj_k(r0, xb)
            proj_qv(r0, xb, jobs[t::NT1], never)
        put_kt(r, kh)
        return c
    x_copy(0).wait()
    qkv_copies[1].wait()
    x_copy(1).start()
    for cp in ffn_copies[0]:
        cp.start()
    xbs = []
    kh0 = []
    NA = 2
    for t in range(NT1):
        x = x_ref[pl.ds(t * TR, TR), :].astype(f32)
        xres[pl.ds(t * TR, TR), :] = x
        xbs.append(_ln(x).astype(bf16))
        if t < NA:
            kh0 += proj_k(t * TR, xbs[t])
    qkv_copies[0].wait()
    qkv_copies[2].wait()
    x_copy(2).start()
    for cp in ffn_copies[1]:
        cp.start()
    wqt[...] = wqkv_ref[0].astype(f32).T.astype(bf16)
    wvt[...] = wqkv_ref[2].astype(f32).T.astype(bf16)
    for t in range(NA, NT1):
        kh0 += proj_k(t * TR, xbs[t])
    for t in range(NT1):
        proj_qv(t * TR, xbs[t])
    put_kt(0, kh0)
    for cp in ffn_copies[0]:
        cp.wait()
    x_copy(3).start()
    for cp in w_copies:
        cp.start()
    lax.fori_loop(1, S // (NT1 * TR), first, 0)

    def set_q(h):
        moff = pl.multiple_of((h % 8) * 8, 8)
        poff = pl.multiple_of(((h + 7) % 8) * 8, 8)
        qm_s[0, pl.ds(poff, 8), :] = jnp.zeros((8, S), u32)
        qm_s[0, pl.ds(moff, 8), :] = qt_s[pl.ds(pl.multiple_of(h * 8, 8), 8), :]

    order, attach, foreign = _plan()
    no = len(order)
    bufof = {x[:2]: ring[i % NR] for i, x in enumerate(order)}

    def head_fast(h, o_prev, main=True):
        g = h // 8
        hp = jnp.maximum(h - 1, 0)
        hpo = jnp.where(h > 0, h - 1, H)
        if main:
            for t in sorted({x[1] // 4 for x in order if x[2]} - {0}):
                prep(h, t)
        zc = [0]

        def zero():
            zc[0] += 1
            return z_s[zc[0] - 1]
        never = zv_s[zero()] != 0
        o = [jnp.zeros((DH, TQ), f32) for _ in range(NB)] + [o_prev]
        l = [[None] * 4 for _ in range(NB)]
        vcnt = {}

        def addl(b, j, v):
            l[b][j] = v if l[b][j] is None else l[b][j] + v

        def do_qk(i):
            b, ci, r0 = order[i]
            z = zero()
            kc = pltpu.bitcast(k_s[g + z, pl.ds((ci * KC + r0) // 2, (KC - r0) // 2), :], bf16)
            qm = pltpu.bitcast(qm_s[z, :, pl.ds(b * TQ, TQ)], bf16)
            p = jnp.exp2(jnp.dot(kc, qm, preferred_element_type=f32))
            nr = (KC - r0) // 8
            p3 = p.reshape(nr, 8, TQ)
            nxt = [0] * 4

            def flush(j, upto):
                if upto > nxt[j]:
                    seg = p3[nxt[j]:upto, :, 128 * j:128 * j + 128]
                    if l[b][j] is not None:
                        seg = jnp.concatenate([l[b][j][None], seg], axis=0)
                    l[b][j] = jnp.sum(seg, axis=0)
                    nxt[j] = upto
            for r in range(nr):
                for j in range(4):
                    for pb, c, a in attach.get((i, r, j), []):
                        flush(j, r + 1)
                        ps = do_vpu(pb, c, a, j)
                        if pb != b:
                            lacc[pb][0, 1 + c * 2 + a, :, pl.ds(j * 128, 128)] = ps
                            l[b][j] = jnp.where(never, ps, l[b][j])
                        else:
                            addl(b, j, ps)
            for j in range(4):
                flush(j, nr)
            for j in range(4):
                bufof[(b, ci)][0, j, pl.ds(r0, KC - r0), :] = p[:, 128 * j:128 * j + 128].astype(bf16)
            if i == no - 1 or order[i + 1][0] != b:
                lacc[b][0, 0] = jnp.concatenate(l[b], axis=-1)

        def do_vpu(b, c, a, j):
            t, sb = divmod(c, 4)
            accs = [None] * NCH
            z = zero()
            hq = h + z
            for d in range(DH):
                if QF:
                    qd = qf_s[hq, pl.ds(d, 1), pl.ds(b * TQ + j * 128, 128)]
                    kbd = kbs[t][z, d, pl.ds(sb * 32 + a * 16, 16), :]
                    tt = qd * kbd
                else:
                    kbd = kbs[t][z, d, pl.ds(sb * 32 + a * 16, 16), :]
                    qd = qf_s[hq, pl.ds(d, 1), pl.ds(b * TQ + j * 128, 128)]
                    tt = kbd * qd
                i2 = d % NCH
                accs[i2] = tt if accs[i2] is None else (tt + accs[i2] if QF == 2 else accs[i2] + tt)
            acc = accs[0]
            for x in accs[1:]:
                acc = acc + x
            p = jnp.exp2(acc)
            bufof[(b, c)][0, j, pl.ds(a * 16, 16), :] = p.astype(bf16)
            vcnt[(b, c)] = vcnt.get((b, c), 0) + 4
            return p[0:8] + p[8:16]
        done = [0] * NB + [NC - LAG]

        def do_pv(i):
            prev = i < 0
            b, ci, r0 = order[i % no]
            assert prev or vcnt.get((b, ci), 0) == r0
            ob = NB if prev else b
            z = zero()
            h8 = pl.multiple_of((hp if prev else h) * 8, 8)
            vt = pltpu.bitcast(vt_s[pl.ds(h8, 8), pl.ds(ci * KC, KC)], bf16)
            o[ob] = o[ob] + jnp.dot(vt, jnp.concatenate([pltpu.bitcast(bufof[(b, ci)].bitcast(u32)[z, j, pl.ds(0, KC // 2), :], bf16) for j in range(4)], axis=1), preferred_element_type=f32)
            done[ob] += 1
            if done[ob] == NC:
                cols = []
                for j in range(4):
                    v = lacc[b][z, 0, :, pl.ds(j * 128, 128)]
                    for sub in foreign[(b, j)]:
                        v = v + lacc[b][z, 1 + sub, :, pl.ds(j * 128, 128)]
                    cols.append(v)
                lsum = jnp.sum(jnp.concatenate(cols, axis=-1), axis=0, keepdims=True)
                hoff = pl.multiple_of((hpo if prev else h) * DH, DH)
                ot_s[pl.ds(hoff, DH), pl.ds(b * TQ, TQ)] = o[ob] * (1.0 / lsum)
        for i in range(no if main else LAG):
            if main:
                do_qk(i)
            do_pv(i - LAG)
        assert zc[0] <= NZ
        if main:
            set_q((h + 1) % H)
            if NPF:
                prep((h + 1) % H, 0)
            return o[NB - 1]

    def head_safe(h, c):
        g = h // 8
        hoff = pl.multiple_of(h * DH, DH)
        h8 = pl.multiple_of(h * 8, 8)
        set_q(h)

        def blk(b, c2):
            q0 = pl.multiple_of(b * TQ, TQ)
            qm = pltpu.bitcast(qm_s[0, :, pl.ds(q0, TQ)], bf16)

            def scores(ci, m):
                kc = pltpu.bitcast(k_s[g, pl.ds(pl.multiple_of(ci * 128, 128), 128), :], bf16)
                s = jnp.dot(kc, qm, preferred_element_type=f32)
                sc_s[pl.ds(pl.multiple_of(ci * 256, 256), 256), :] = s
                return jnp.maximum(m, jnp.max(s.reshape(32, 8, TQ), axis=0))
            m = lax.fori_loop(0, S // 256, scores, jnp.full((8, TQ), -jnp.inf, f32))
            m = jnp.max(m, axis=0, keepdims=True)

            def accum(ci, lo):
                c0 = pl.multiple_of(ci * 256, 256)
                p = jnp.exp2(sc_s[pl.ds(c0, 256), :] - m)
                vt = pltpu.bitcast(vt_s[pl.ds(h8, 8), pl.ds(c0, 256)], bf16)
                return (lo[0] + jnp.sum(p.reshape(32, 8, TQ), axis=0),
                        lo[1] + jnp.dot(vt, p.astype(bf16), preferred_element_type=f32))
            l, o = lax.fori_loop(0, S // 256, accum, (jnp.zeros((8, TQ), f32), jnp.zeros((DH, TQ), f32)))
            ot_s[pl.ds(hoff, DH), pl.ds(q0, TQ)] = o * (1.0 / jnp.sum(l, axis=0, keepdims=True))
            return c2
        lax.fori_loop(0, NB, blk, 0)
        return c

    def attention():
        qn = jnp.max(st_s[0], axis=1, keepdims=True)
        kn = jnp.max(st_s[1], axis=1, keepdims=True)
        bound2 = jnp.max(qn * kn) * 1.05
        vmax = jnp.max(st_s[2])
        st_s[...] = jnp.zeros_like(st_s)
        ok = jnp.logical_and(bound2 <= SAFE_LOG2 * SAFE_LOG2,
                             jnp.logical_and(vmax <= 2.0 ** 40, vmax >= 2.0 ** -30))

        @pl.when(ok)
        def _():
            set_q(0)
            o_last = lax.fori_loop(0, H, head_fast, jnp.zeros((DH, TQ), f32))
            head_fast(H, o_last, main=False)

        @pl.when(jnp.logical_not(ok))
        def _():
            lax.fori_loop(0, H, head_safe, 0)

    def dense(last):
        nt = NT3 if last else NT2

        def body(r, c):
            r0s = [pl.multiple_of(r * (nt * TR) + t * TR, TR) for t in range(nt)]
            if not last:
                prep(0, 0)
            xs = []
            for t in range(0, nt, 2):
                o1 = ot_s[pl.ds(0, D), pl.ds(r0s[t], TR)].T
                o2 = ot_s[pl.ds(0, D), pl.ds(r0s[t + 1], TR)].T
                if SWO:
                    cs = _strassen(_lhs_combos(o1, o2, D // 2), woc, CW, z_s[t])
                    a1, a2 = jnp.concatenate(cs[:2], axis=1), jnp.concatenate(cs[2:], axis=1)
                else:
                    a1 = jnp.dot(o1.astype(bf16), wo_ref[...], preferred_element_type=f32)
                    a2 = jnp.dot(o2.astype(bf16), wo_ref[...], preferred_element_type=f32)
                xs.append(xres[pl.ds(r0s[t], TR), :] + a1)
                xs.append(xres[pl.ds(r0s[t + 1], TR), :] + a2)
            hs = []
            for t in range(0, nt, 2):
                n1, n2 = _ln(xs[t]), _ln(xs[t + 1])
                if SF1:
                    cs = _strassen(_lhs_combos(n1, n2, D // 2), w1c, CW1, z_s[t])
                    h1, h2 = cs[:2], cs[2:]
                    if 2 * FH < F:
                        h1.append(jnp.dot(n1.astype(bf16), w1_ref[:, 2 * FH:F], preferred_element_type=f32))
                        h2.append(jnp.dot(n2.astype(bf16), w1_ref[:, 2 * FH:F], preferred_element_type=f32))
                    h1, h2 = jnp.concatenate(h1, axis=1), jnp.concatenate(h2, axis=1)
                else:
                    h1 = jnp.dot(n1.astype(bf16), w1_ref[...], preferred_element_type=f32)
                    h2 = jnp.dot(n2.astype(bf16), w1_ref[...], preferred_element_type=f32)
                h1, h2 = _gelu(h1 + bias_s[0:1, 0:F]), _gelu(h2 + bias_s[0:1, 0:F])
                if SF2:
                    hs.append((_lhs_combos(h1, h2, FH), h1[:, 2 * FH:F].astype(bf16), h2[:, 2 * FH:F].astype(bf16)))
                else:
                    hs.append((h1.astype(bf16), h2.astype(bf16)))
            ds = []
            for t, hh in enumerate(hs):
                if SF2:
                    cs = _strassen(hh[0], w2c, CW, z_s[t])
                    d1, d2 = jnp.concatenate(cs[:2], axis=1), jnp.concatenate(cs[2:], axis=1)
                    if 2 * FH < F:
                        d1 = d1 + jnp.dot(hh[1], w2_ref[2 * FH:F, :], preferred_element_type=f32)
                        d2 = d2 + jnp.dot(hh[2], w2_ref[2 * FH:F, :], preferred_element_type=f32)
                else:
                    d1 = jnp.dot(hh[0], w2_ref[...], preferred_element_type=f32)
                    d2 = jnp.dot(hh[1], w2_ref[...], preferred_element_type=f32)
                ds += [d1, d2]
            kh = []
            ys = []
            for t in range(nt):
                x = xs[t] + ds[t] + bias_s[1:2, 0:D]
                ys.append(x)
                if last:
                    x_ref[pl.ds(r0s[t], TR), :] = x.astype(bf16)
                    if ((t + 1) * TR) % TO == 0:
                        o_copy(r * (nt * TR // TO) + (t + 1) * TR // TO - 1).start()
            if not last:
                for r0, x in zip(r0s, ys):
                    xres[pl.ds(r0, TR), :] = x
                for t in range(0, nt, 2):
                    kh += proj2(r0s[t], ys[t], r0s[t + 1], ys[t + 1], z_s[t])
                put_kt(r, kh)
            return c
        lax.fori_loop(0, S // (nt * TR), body, 0)

    def layer(i, c):
        attention()

        @pl.when(i == 0)
        def _():
            for cp in w_copies:
                cp.wait()
            bias_s[0:1, 0:F] = b1_ref[pl.ds(0, F)].astype(f32)[None, :]
            bias_s[1:2, 0:D] = b2_ref[pl.ds(0, D)].astype(f32)[None, :]
            dense(False)

        @pl.when(i == 1)
        def _():
            dense(True)
        return c
    lax.fori_loop(0, 2, layer, 0)
    for r in range(S // TO):
        o_copy(r).wait()


@jax.jit
def pallas_interleave_layers__mha_block__dense_activation_gelu__prompt_kernel(A_x, A_wqkv, A_wo, B_x, B_w1, B_b1, B_w2, B_b2):
    x = A_x.reshape(S, D)
    hbm = pl.BlockSpec(memory_space=pl.ANY)
    out = pl.pallas_call(
        _kernel,
        out_shape=jax.ShapeDtypeStruct((S, D), bf16),
        in_specs=[hbm] * 7,
        out_specs=hbm,
        scratch_shapes=[
            pltpu.VMEM((S, D), bf16),
            pltpu.VMEM((3, D, D), bf16),
            pltpu.VMEM((D, D), bf16),
            pltpu.VMEM((D, F), bf16),
            pltpu.VMEM((F, D), bf16),
            pltpu.SemaphoreType.DMA((S // TI,)),
            pltpu.SemaphoreType.DMA((14,)),
            pltpu.SemaphoreType.DMA((S // TO,)),
            pltpu.VMEM((S, D), f32),
            pltpu.VMEM((D, D), bf16),
            pltpu.VMEM((D, D), bf16),
            pltpu.VMEM((4, S // 2, 128), u32),
            pltpu.VMEM((D // 2, S), u32),
            pltpu.VMEM((D // 2, S), u32),
            pltpu.VMEM((H, DH, S + QPAD), f32),
            pltpu.VMEM((4, H, DH, 128), f32),
            pltpu.VMEM((D + DH, S), f32),
            pltpu.VMEM((1, 64, S), u32),
            pltpu.VMEM((3, H, TR), f32),
            pltpu.VMEM((S, TQ), f32),
            pltpu.VMEM((4, 8, 128), jnp.int32),
            pltpu.VMEM((8, 2048), f32),
            pltpu.SMEM((NZ,), jnp.int32),
        ] + [pltpu.VMEM((1, 4, KC + RPAD, 128), bf16) for _ in range(NR)]
          + [pltpu.VMEM((1, DH, 128 + KPAD, 128), f32) for _ in range(NVM)]
          + [pltpu.VMEM((1, NL, 8, TQ), f32) for _ in range(NB)]
          + [pltpu.VMEM((8192,), bf16), pltpu.VMEM((8192,), bf16),
             pltpu.VMEM((7, D // 4, FH), u32), pltpu.VMEM((7, FH // 2, D // 2), u32), pltpu.VMEM((7, D // 4, D // 2), u32),
             pltpu.VMEM((7, D // 4, D // 2), u32), pltpu.VMEM((7, D // 2, D // 2), u32)],
        compiler_params=pltpu.CompilerParams(vmem_limit_bytes=100 * 2 ** 20),
    )(x, A_wqkv, A_wo, B_w1, B_b1, B_w2, B_b2)
    return out.reshape(1, S, D)
```

```python
import jax
import jax.numpy as jnp
from jax import lax
import jax.experimental.pallas as pl
import jax.experimental.pallas.tpu as pltpu

S, D, H, DH, F = 2048, 512, 32, 16, 1792
TR = 128
NT = 4
TI = NT * TR
TQ = 512
KC = 128
NB = S // TQ
NC = S // KC
HD = D // 2
FH = F // 2

LAG = 4
NR = 16
NP0 = (3.5, 0, 0, 0)
NS = (5, 9, 10.5, 9)
START = 8
PVM = 2
RPS = 14
W1 = 0.9
Z1 = 170
W2 = 0.95
Z2 = 90
KPAD = 8
RPAD = 16
NL = 36
NZ = 600

QSCALE = (DH ** -0.5) * 1.4426950408889634
SAFE_LOG2 = 60.0
bf16 = jnp.bfloat16
f32 = jnp.float32
u32 = jnp.uint32
NT_DIMS = (((1,), (1,)), ((), ()))


def _ln(x):
    m = jnp.mean(x, axis=-1, keepdims=True)
    xc = x - m
    v = jnp.mean(xc * xc, axis=-1, keepdims=True)
    return xc * lax.rsqrt(v + 1e-5)


def _gelu(x):
    c = 0.7978845608028654
    return 0.5 * x * (1.0 + jnp.tanh(c * (x + 0.044715 * (x * x * x))))


def _pack(x):
    return pltpu.bitcast(x.astype(bf16), u32)


def _unpack(x):
    return pltpu.bitcast(x, bf16)


def _lhs_combos(a1, a2):
    kh = a1.shape[1] // 2
    a11, a12, a21, a22 = a1[:, :kh], a1[:, kh:], a2[:, :kh], a2[:, kh:]
    return [t.astype(bf16) for t in (a11 + a22, a21 + a22, a11, a22, a11 + a12, a21 - a11, a12 - a22)]


def _rhs_jobs(w_ref, c_ref, part, transposed=False, row0=0):
    kh, nh = w_ref.shape[0] // 2, w_ref.shape[1] // 2
    units = kh // 16
    per = -(-units // 3)
    start = jnp.minimum(part * per, units - per)

    def job(u, c0, w):
        def run():
            r = pl.multiple_of((start + u) * 16, 16)
            b11, b12, b21, b22 = (w_ref[pl.ds(rr, 16), pl.ds(cc, w)].astype(f32)
                                  for rr in (r, kh + r) for cc in (c0, nh + c0))
            if transposed:
                b12, b21 = b21, b12
            r2 = pl.multiple_of(row0 + (start + u) * 8, 8)
            tok = None
            for n, t in enumerate((b11 + b22, b11, b12 - b22, b21 - b11, b22, b11 + b12, b21 + b22)):
                t = _pack(t)
                c_ref[n, pl.ds(r2, 8), pl.ds(c0, w)] = t
                for l0 in range(0, w, 128):
                    tok = t[:, l0:l0 + 128] if tok is None else tok | t[:, l0:l0 + 128]
            return pltpu.bitcast(tok, f32)
        return run
    return [job(u, c0, min(256, nh - c0)) for u in range(per) for c0 in range(0, nh, 256)]


def _strassen(ac, c_ref, cw, z):
    out = [[], [], [], []]
    for c0 in range(0, c_ref.shape[2], cw):
        def m(i):
            return jnp.dot(ac[i], _unpack(c_ref[i + z, :, c0:c0 + cw]), preferred_element_type=f32)
        m2, m4 = m(1), m(3)
        out[2].append(m2 + m4)
        m1 = m(0)
        t11, t22 = m1 + m4, m1 - m2
        m3 = m(2)
        t22 = t22 + m3
        m5 = m(4)
        out[1].append(m3 + m5)
        out[0].append(t11 - m5 + m(6))
        out[3].append(t22 + m(5))
    return jnp.concatenate(out[0] + out[1], axis=1), jnp.concatenate(out[2] + out[3], axis=1)


def _strassen_t(ac, c_ref, row0, z):
    def m(i):
        return lax.dot_general(_unpack(c_ref[i + z, row0:row0 + HD // 2, :]), ac[i], NT_DIMS,
                               preferred_element_type=f32)
    m2, m4 = m(1), m(3)
    c21 = m2 + m4
    m1, m3 = m(0), m(2)
    t11, t22 = m1 + m4, m1 - m2 + m3
    m5 = m(4)
    c12 = m3 + m5
    c11 = t11 - m5 + m(6)
    c22 = t22 + m(5)
    return jnp.concatenate([c11, c12], axis=0), jnp.concatenate([c21, c22], axis=0)


def _plan():
    def groups(first, n):
        out = [(first + i, 32) for i in range(int(n))]
        return out + [(first + int(n), 16)] * (n != int(n))
    subs = [groups(0, m) + groups(4, n) for m, n in zip(NP0, NS)]
    nrows = sum(NC * 16 - sum(r // 8 for _, r in x) for x in subs)
    pieces = [(b, c, a, j) for b in range(NB) for c, r in subs[b] for a in range(r // 16) for j in range(4)]
    wts = [0.0 if r < START else W1 if r < Z1 else W2 if r >= nrows - Z2 else 1.0 for r in range(nrows)]
    pos = {}
    row, cum = 0, 0.0
    for k, pc in enumerate(pieces):
        while cum + wts[row] <= (k + 0.5) * sum(wts) / len(pieces):
            cum += wts[row]
            row += 1
        pos[pc] = row
    order = []
    row = 0
    for b in range(NB):
        mixed = list(subs[b])
        pure = [c for c in range(NC) if c not in dict(mixed)]
        while mixed or pure:
            if mixed and (not pure or row + (LAG - PVM) * RPS > pos[(b, mixed[0][0], mixed[0][1] // 16 - 1, 3)]):
                order.append((b,) + mixed.pop(0))
            else:
                order.append((b, pure.pop(0), 0))
            row += 16 - order[-1][2] // 8
    rows = [(i, r) for i, x in enumerate(order) for r in range(16 - x[2] // 8)]
    step_of = {x[:2]: i for i, x in enumerate(order)}
    attach = {}
    foreign = {(b, j): [] for b in range(NB) for j in range(4)}
    for (pb, c, a, j), p in pos.items():
        i, r = rows[p]
        assert step_of[(pb, c)] - NR + LAG < i <= step_of[(pb, c)] + LAG
        assert pb < NB - 1 or i >= LAG
        attach.setdefault((i, r, j), []).append((pb, c, a))
        if pb != order[i][0]:
            foreign[(pb, j)].append(c * 2 + a)
    return order, attach, foreign


def _kernel(x_hbm, wqkv_hbm, wo_hbm, w1_hbm, b1_hbm, w2_hbm, b2_hbm, o_hbm,
            x_ref, wqkv_ref, wo_ref, w1_ref, w2_ref, sem_x, sem_w, sem_o,
            xres, wqt, wvt, k_s, qt_s, vt_s, qf_s, kt_s, ot_s, qm_s, st_s, sc_s, zv_s, bias_s, z_s, *bufs):
    ring = bufs[:NR]
    kbs = bufs[NR:NR + 4]
    lacc = bufs[NR + 4:NR + 4 + NB]
    b1_ref, b2_ref, w1c, w2c, wkc, wqvc, wot = bufs[NR + 4 + NB:]

    def x_copy(r):
        rows = pl.ds(pl.multiple_of(r * TI, TI), TI)
        return pltpu.make_async_copy(x_hbm.at[rows], x_ref.at[rows], sem_x.at[r])

    def o_copy(r):
        rows = pl.ds(pl.multiple_of(r * TR, TR), TR)
        return pltpu.make_async_copy(x_ref.at[rows], o_hbm.at[rows], sem_o.at[r])
    b_copies = [pltpu.make_async_copy(b1_hbm, b1_ref.at[pl.ds(0, F)], sem_w.at[0]),
                pltpu.make_async_copy(b2_hbm, b2_ref.at[pl.ds(0, D)], sem_w.at[1])]
    qkv_copies = [pltpu.make_async_copy(wqkv_hbm.at[:, pl.ds(i * D, D)], wqkv_ref.at[i], sem_w.at[3 + i])
                  for i in range(3)]
    w_copies = [[], []]
    for src, dst in ((w1_hbm, w1_ref), (w2_hbm, w2_ref)):
        kh = src.shape[0] // 2
        cut = -(-(kh // 16) // 3) * 16
        for half in (0, kh):
            for stage, rows in enumerate((pl.ds(half, cut), pl.ds(half + cut, kh - cut))):
                sem = sem_w.at[6 + len(w_copies[0]) + len(w_copies[1])]
                w_copies[stage].append(pltpu.make_async_copy(src.at[rows], dst.at[rows], sem))
    w_copies[0].append(pltpu.make_async_copy(wo_hbm.at[pl.ds(0, HD)], wo_ref.at[pl.ds(0, HD)], sem_w.at[2]))
    w_copies[1].append(pltpu.make_async_copy(wo_hbm.at[pl.ds(HD, HD)], wo_ref.at[pl.ds(HD, HD)], sem_w.at[14]))
    x_copy(0).start()
    qkv_copies[1].start()

    qm_s[...] = jnp.zeros_like(qm_s)
    st_s[...] = jnp.zeros_like(st_s)
    zv_s[...] = jnp.zeros_like(zv_s)
    for buf in ring[NR - LAG:]:
        buf[...] = jnp.zeros_like(buf)
    lacc[NB - 1][...] = jnp.ones_like(lacc[NB - 1])
    for i in range(NZ):
        z_s[i] = 0

    def put_k(r0, k):
        kp = _pack(k)
        r2 = pl.multiple_of(r0 // 2, TR // 2)
        for g in range(4):
            k_s[g, pl.ds(r2, TR // 2), :] = kp[:, g * 128:(g + 1) * 128]
        kt = k.T.reshape(H, DH, TR)
        st_s[1] = jnp.maximum(st_s[1], jnp.sum(kt * kt, axis=1))
        return k[0:32]

    def put_qv(r0, q, v):
        q = q * QSCALE
        qt_s[:, pl.ds(r0, TR)] = _pack(q)
        q3 = q.reshape(H, DH, TR)
        qf_s[:, :, pl.ds(r0, TR)] = q3
        vt_s[:, pl.ds(r0, TR)] = _pack(v)
        st_s[0] = jnp.maximum(st_s[0], jnp.sum(q3 * q3, axis=1))
        st_s[2] = jnp.maximum(st_s[2], jnp.max(jnp.abs(v).reshape(DH, H, TR), axis=0))

    def put_kt(r, heads):
        kt_s[r] = jnp.concatenate(heads, axis=0).T.reshape(H, DH, 128)

    def proj_k(r0, xb):
        return put_k(r0, jnp.dot(xb, wqkv_ref[1], preferred_element_type=f32))

    def proj_qv(r0, xb, jobs=(), never=None):
        out = []
        for n, w in enumerate((wqt, wvt)):
            y = lax.dot_general(w[...], xb, NT_DIMS, preferred_element_type=f32)
            mine = jobs[n::2]
            if mine:
                step = D // len(mine) // 8 * 8
                parts = []
                for i, run in enumerate(mine):
                    parts.append(jnp.where(never, run(), y[i * step:i * step + 8]))
                    parts.append(y[i * step + 8:(i + 1) * step if i + 1 < len(mine) else D])
                y = jnp.concatenate(parts, axis=0)
            out.append(y)
        put_qv(r0, *out)

    def proj_pair(r1, x1, r2, x2, z):
        ac = _lhs_combos(_ln(x1), _ln(x2))
        k1, k2 = _strassen(ac, wkc, 128, z)
        kh = [put_k(r1, k1), put_k(r2, k2)]
        q1, q2 = _strassen_t(ac, wqvc, 0, z)
        v1, v2 = _strassen_t(ac, wqvc, HD // 2, z)
        put_qv(r1, q1, v1)
        put_qv(r2, q2, v2)
        return kh

    def prep(h, t):
        for d in range(DH):
            row = jnp.broadcast_to(kt_s[t, h, pl.ds(d, 1), :], (128, 128))
            kbs[t][0, d, pl.ds(0, 128), :] = row.T

    def load_x(r0):
        x = x_ref[pl.ds(r0, TR), :].astype(f32)
        xres[pl.ds(r0, TR), :] = x
        return _ln(x).astype(bf16)

    def first(r, c):
        @pl.when(r == 2)
        def _():
            for cp in w_copies[1]:
                cp.wait()
        x_copy(r).wait()
        prep(0, 0)
        never = zv_s[z_s[0]] != 0
        jobs = (_rhs_jobs(w1_ref, w1c, r - 1) + _rhs_jobs(w2_ref, w2c, r - 1)
                + _rhs_jobs(wqkv_ref.at[1], wkc, r - 1) + _rhs_jobs(wqt, wqvc, r - 1, True)
                + _rhs_jobs(wvt, wqvc, r - 1, True, HD // 2))

        def wo_job(u):
            def run():
                c0 = pl.multiple_of((r - 1 + u) * 128, 128)
                y = wo_ref[pl.ds(c0, 128), :].astype(f32).T
                wot[:, pl.ds(c0, 128)] = y.astype(bf16)
                return jnp.max(y.reshape(D // 8, 8, 128), axis=0)
            return run
        jobs = jobs[:30] + [wo_job(0)] + jobs[30:50] + [wo_job(1)] + jobs[50:]
        kh = []
        for t in range(NT):
            r0 = pl.multiple_of(r * TI + t * TR, TR)
            xb = load_x(r0)
            kh.append(proj_k(r0, xb))
            proj_qv(r0, xb, jobs[t::NT], never)
        put_kt(r, kh)
        return c

    x_copy(0).wait()
    qkv_copies[0].start()
    qkv_copies[2].start()
    xbs = [load_x(0)]
    qkv_copies[1].wait()
    x_copy(1).start()
    for cp in w_copies[0]:
        cp.start()
    xbs += [load_x(t * TR) for t in range(1, NT)]
    kh0 = [proj_k(t * TR, xbs[t]) for t in range(NT - 1)]
    qkv_copies[0].wait()
    qkv_copies[2].wait()
    x_copy(2).start()
    for cp in w_copies[1]:
        cp.start()
    wqt[...] = wqkv_ref[0].astype(f32).T.astype(bf16)
    wvt[...] = wqkv_ref[2].astype(f32).T.astype(bf16)
    kh0.append(proj_k((NT - 1) * TR, xbs[NT - 1]))
    for t in range(NT):
        proj_qv(t * TR, xbs[t])
    put_kt(0, kh0)
    for cp in w_copies[0]:
        cp.wait()
    x_copy(3).start()
    for cp in b_copies:
        cp.start()
    lax.fori_loop(1, S // TI, first, 0)

    def set_q(h):
        moff = pl.multiple_of((h % 8) * 8, 8)
        poff = pl.multiple_of(((h + 7) % 8) * 8, 8)
        qm_s[0, pl.ds(poff, 8), :] = jnp.zeros((8, S), u32)
        qm_s[0, pl.ds(moff, 8), :] = qt_s[pl.ds(pl.multiple_of(h * 8, 8), 8), :]

    order, attach, foreign = _plan()
    no = len(order)
    bufof = {x[:2]: ring[i % NR] for i, x in enumerate(order)}

    def head_fast(h, o_prev, main=True):
        g = h // 8
        hp = jnp.maximum(h - 1, 0)
        hpo = jnp.where(h > 0, h - 1, H)
        if main:
            for t in sorted({x[1] // 4 for x in order if x[2]} - {0}):
                prep(h, t)
        zc = [0]

        def zero():
            zc[0] += 1
            return z_s[zc[0] - 1]
        never = zv_s[zero()] != 0
        o = [jnp.zeros((DH, TQ), f32) for _ in range(NB)] + [o_prev]
        l = [[None] * 4 for _ in range(NB)]

        def do_vpu(b, c, a, j):
            t, sb = divmod(c, 4)
            acc = [None, None]
            z = zero()
            hq = h + z
            for d in range(DH):
                kbd = kbs[t][z, d, pl.ds(sb * 32 + a * 16, 16), :]
                qd = qf_s[hq, pl.ds(d, 1), pl.ds(b * TQ + j * 128, 128)]
                tt = kbd * qd
                acc[d % 2] = tt if acc[d % 2] is None else acc[d % 2] + tt
            p = jnp.exp2(acc[0] + acc[1])
            bufof[(b, c)][0, j, pl.ds(a * 16, 16), :] = p.astype(bf16)
            return p[0:8] + p[8:16]

        def do_qk(i):
            b, ci, r0 = order[i]
            z = zero()
            kc = _unpack(k_s[g + z, pl.ds((ci * KC + r0) // 2, (KC - r0) // 2), :])
            qm = _unpack(qm_s[z, :, pl.ds(b * TQ, TQ)])
            p = jnp.exp2(jnp.dot(kc, qm, preferred_element_type=f32))
            nr = (KC - r0) // 8
            p3 = p.reshape(nr, 8, TQ)
            nxt = [0] * 4

            def flush(j, upto):
                if upto > nxt[j]:
                    seg = p3[nxt[j]:upto, :, 128 * j:128 * j + 128]
                    if l[b][j] is not None:
                        seg = jnp.concatenate([l[b][j][None], seg], axis=0)
                    l[b][j] = jnp.sum(seg, axis=0)
                    nxt[j] = upto
            for r in range(nr):
                for j in range(4):
                    for pb, c, a in attach.get((i, r, j), []):
                        flush(j, r + 1)
                        ps = do_vpu(pb, c, a, j)
                        if pb != b:
                            lacc[pb][0, 1 + c * 2 + a, :, pl.ds(j * 128, 128)] = ps
                            l[b][j] = jnp.where(never, ps, l[b][j])
                        else:
                            l[b][j] = l[b][j] + ps
            for j in range(4):
                flush(j, nr)
            for j in range(4):
                bufof[(b, ci)][0, j, pl.ds(r0, KC - r0), :] = p[:, 128 * j:128 * j + 128].astype(bf16)
            if i == no - 1 or order[i + 1][0] != b:
                lacc[b][0, 0] = jnp.concatenate(l[b], axis=-1)
        done = [0] * NB + [NC - LAG]

        def do_pv(i):
            prev = i < 0
            b, ci, _ = order[i % no]
            ob = NB if prev else b
            z = zero()
            h8 = pl.multiple_of((hp if prev else h) * 8, 8)
            vt = _unpack(vt_s[pl.ds(h8, 8), pl.ds(ci * KC, KC)])
            words = bufof[(b, ci)].bitcast(u32)
            p = jnp.concatenate([_unpack(words[z, j, pl.ds(0, KC // 2), :]) for j in range(4)], axis=1)
            o[ob] = o[ob] + jnp.dot(vt, p, preferred_element_type=f32)
            done[ob] += 1
            if done[ob] == NC:
                cols = []
                for j in range(4):
                    v = lacc[b][z, 0, :, pl.ds(j * 128, 128)]
                    for sub in foreign[(b, j)]:
                        v = v + lacc[b][z, 1 + sub, :, pl.ds(j * 128, 128)]
                    cols.append(v)
                lsum = jnp.sum(jnp.concatenate(cols, axis=-1), axis=0, keepdims=True)
                hoff = pl.multiple_of((hpo if prev else h) * DH, DH)
                ot_s[pl.ds(hoff, DH), pl.ds(b * TQ, TQ)] = o[ob] * (1.0 / lsum)
        for i in range(no if main else LAG):
            if main:
                do_qk(i)
            do_pv(i - LAG)
        assert zc[0] <= NZ
        if main:
            set_q((h + 1) % H)
            prep((h + 1) % H, 0)
            return o[NB - 1]

    def head_safe(h, c):
        g = h // 8
        hoff = pl.multiple_of(h * DH, DH)
        h8 = pl.multiple_of(h * 8, 8)
        set_q(h)

        def blk(b, c2):
            q0 = pl.multiple_of(b * TQ, TQ)
            qm = _unpack(qm_s[0, :, pl.ds(q0, TQ)])

            def scores(ci, m):
                kc = _unpack(k_s[g, pl.ds(pl.multiple_of(ci * 128, 128), 128), :])
                s = jnp.dot(kc, qm, preferred_element_type=f32)
                sc_s[pl.ds(pl.multiple_of(ci * 256, 256), 256), :] = s
                return jnp.maximum(m, jnp.max(s.reshape(32, 8, TQ), axis=0))
            m = lax.fori_loop(0, S // 256, scores, jnp.full((8, TQ), -jnp.inf, f32))
            m = jnp.max(m, axis=0, keepdims=True)

            def accum(ci, lo):
                c0 = pl.multiple_of(ci * 256, 256)
                p = jnp.exp2(sc_s[pl.ds(c0, 256), :] - m)
                vt = _unpack(vt_s[pl.ds(h8, 8), pl.ds(c0, 256)])
                return (lo[0] + jnp.sum(p.reshape(32, 8, TQ), axis=0),
                        lo[1] + jnp.dot(vt, p.astype(bf16), preferred_element_type=f32))
            l, o = lax.fori_loop(0, S // 256, accum, (jnp.zeros((8, TQ), f32), jnp.zeros((DH, TQ), f32)))
            ot_s[pl.ds(hoff, DH), pl.ds(q0, TQ)] = o * (1.0 / jnp.sum(l, axis=0, keepdims=True))
            return c2
        lax.fori_loop(0, NB, blk, 0)
        return c

    def attention():
        qn = jnp.max(st_s[0], axis=1, keepdims=True)
        kn = jnp.max(st_s[1], axis=1, keepdims=True)
        bound2 = jnp.max(qn * kn) * 1.05
        vmax = jnp.max(st_s[2])
        st_s[...] = jnp.zeros_like(st_s)
        ok = jnp.logical_and(bound2 <= SAFE_LOG2 * SAFE_LOG2,
                             jnp.logical_and(vmax <= 2.0 ** 40, vmax >= 2.0 ** -30))

        @pl.when(ok)
        def _():
            set_q(0)
            o_last = lax.fori_loop(0, H, head_fast, jnp.zeros((DH, TQ), f32))
            head_fast(H, o_last, main=False)

        @pl.when(jnp.logical_not(ok))
        def _():
            lax.fori_loop(0, H, head_safe, 0)

    def dense(last):
        def body(r, c):
            r0s = [pl.multiple_of(r * TI + t * TR, TR) for t in range(NT)]
            if not last:
                prep(0, 0)
            xs = []
            for t, r0 in enumerate(r0s):
                ot = ot_s[pl.ds(0, D), pl.ds(r0, TR)]
                if t == 0:
                    a = jnp.dot(wot[...], ot.astype(bf16), preferred_element_type=f32).T
                else:
                    a = jnp.dot(ot.T.astype(bf16), wo_ref[...], preferred_element_type=f32)
                xs.append(xres[pl.ds(r0, TR), :] + a)
            hs = []
            for t in range(0, NT, 2):
                h1, h2 = _strassen(_lhs_combos(_ln(xs[t]), _ln(xs[t + 1])), w1c, 128, z_s[t])
                hs.append(_lhs_combos(_gelu(h1 + bias_s[0:1, 0:F]), _gelu(h2 + bias_s[0:1, 0:F])))
            ds = []
            for t, hc in enumerate(hs):
                ds += _strassen(hc, w2c, 256, z_s[t])
            ys = []
            for t in range(NT):
                ys.append(xs[t] + ds[t] + bias_s[1:2, 0:D])
                if last:
                    x_ref[pl.ds(r0s[t], TR), :] = ys[t].astype(bf16)
                    o_copy(r * NT + t).start()
            if not last:
                for r0, x in zip(r0s, ys):
                    xres[pl.ds(r0, TR), :] = x
                kh = []
                for t in range(0, NT, 2):
                    kh += proj_pair(r0s[t], ys[t], r0s[t + 1], ys[t + 1], z_s[t])
                put_kt(r, kh)
            return c
        lax.fori_loop(0, S // TI, body, 0)

    def layer(i, c):
        attention()

        @pl.when(i == 0)
        def _():
            for cp in b_copies:
                cp.wait()
            bias_s[0:1, 0:F] = b1_ref[pl.ds(0, F)].astype(f32)[None, :]
            bias_s[1:2, 0:D] = b2_ref[pl.ds(0, D)].astype(f32)[None, :]
            dense(False)

        @pl.when(i == 1)
        def _():
            dense(True)
        return c
    lax.fori_loop(0, 2, layer, 0)
    for r in range(S // TR):
        o_copy(r).wait()


@jax.jit
def pallas_interleave_layers__mha_block__dense_activation_gelu__prompt_kernel(A_x, A_wqkv, A_wo, B_x, B_w1, B_b1, B_w2, B_b2):
    hbm = pl.BlockSpec(memory_space=pl.ANY)
    out = pl.pallas_call(
        _kernel,
        out_shape=jax.ShapeDtypeStruct((S, D), bf16),
        in_specs=[hbm] * 7,
        out_specs=hbm,
        scratch_shapes=[
            pltpu.VMEM((S, D), bf16),
            pltpu.VMEM((3, D, D), bf16),
            pltpu.VMEM((D, D), bf16),
            pltpu.VMEM((D, F), bf16),
            pltpu.VMEM((F, D), bf16),
            pltpu.SemaphoreType.DMA((S // TI,)),
            pltpu.SemaphoreType.DMA((15,)),
            pltpu.SemaphoreType.DMA((S // TR,)),
            pltpu.VMEM((S, D), f32),
            pltpu.VMEM((D, D), bf16),
            pltpu.VMEM((D, D), bf16),
            pltpu.VMEM((4, S // 2, 128), u32),
            pltpu.VMEM((D // 2, S), u32),
            pltpu.VMEM((D // 2, S), u32),
            pltpu.VMEM((H, DH, S), f32),
            pltpu.VMEM((4, H, DH, 128), f32),
            pltpu.VMEM((D + DH, S), f32),
            pltpu.VMEM((1, 64, S), u32),
            pltpu.VMEM((3, H, TR), f32),
            pltpu.VMEM((S, TQ), f32),
            pltpu.VMEM((4, 8, 128), jnp.int32),
            pltpu.VMEM((8, 2048), f32),
            pltpu.SMEM((NZ,), jnp.int32),
        ] + [pltpu.VMEM((1, 4, KC + RPAD, 128), bf16) for _ in range(NR)]
          + [pltpu.VMEM((1, DH, 128 + KPAD, 128), f32) for _ in range(4)]
          + [pltpu.VMEM((1, NL, 8, TQ), f32) for _ in range(NB)]
          + [pltpu.VMEM((8192,), bf16), pltpu.VMEM((8192,), bf16),
             pltpu.VMEM((7, HD // 2, FH), u32), pltpu.VMEM((7, FH // 2, HD), u32),
             pltpu.VMEM((7, HD // 2, HD), u32), pltpu.VMEM((7, HD, HD), u32),
             pltpu.VMEM((D, D), bf16)],
        compiler_params=pltpu.CompilerParams(vmem_limit_bytes=100 * 2 ** 20),
    )(A_x.reshape(S, D), A_wqkv, A_wo, B_w1, B_b1, B_w2, B_b2)
    return out.reshape(1, S, D)
```

```python
import jax
import jax.numpy as jnp
from jax import lax
import jax.experimental.pallas as pl
import jax.experimental.pallas.tpu as pltpu

S, D, H, DH, F = 2048, 512, 32, 16, 1792
TR = 128
NT = 4
TI = NT * TR
TQ = 512
KC = 128
NB = S // TQ
NC = S // KC
HD = D // 2
FH = F // 2

LAG = 4
NR = 16
NP0 = (3.5, 0, 0, 0)
NS = (5, 9, 10.5, 9)
START = 8
PVM = 2
RPS = 14
W1 = 0.9
Z1 = 170
W2 = 0.95
Z2 = 90
KPAD = 8
RPAD = 16
NL = 36
NZ = 600

QSCALE = (DH ** -0.5) * 1.4426950408889634
SAFE_LOG2 = 60.0
bf16 = jnp.bfloat16
f32 = jnp.float32
u32 = jnp.uint32
NT_DIMS = (((1,), (1,)), ((), ()))


def _ln(x):
    m = jnp.mean(x, axis=-1, keepdims=True)
    xc = x - m
    v = jnp.mean(xc * xc, axis=-1, keepdims=True)
    return xc * lax.rsqrt(v + 1e-5)


def _gelu(x):
    c = 0.7978845608028654
    return 0.5 * x * (1.0 + jnp.tanh(c * (x + 0.044715 * (x * x * x))))


def _recip(x):
    r = pl.reciprocal(x, approx=True)
    return r * (2.0 - x * r)


def _pack(x):
    return pltpu.bitcast(x.astype(bf16), u32)


def _unpack(x):
    return pltpu.bitcast(x, bf16)


def _lhs_combos(a1, a2):
    kh = a1.shape[1] // 2
    a11, a12, a21, a22 = a1[:, :kh], a1[:, kh:], a2[:, :kh], a2[:, kh:]
    return [t.astype(bf16) for t in (a11 + a22, a21 + a22, a11, a22, a11 + a12, a21 - a11, a12 - a22)]


def _rhs_jobs(w_ref, c_ref, part, transposed=False, row0=0):
    kh, nh = w_ref.shape[0] // 2, w_ref.shape[1] // 2
    units = kh // 16
    per = -(-units // 3)
    start = jnp.minimum(part * per, units - per)

    def job(u, c0, w):
        def run():
            r = pl.multiple_of((start + u) * 16, 16)
            b11, b12, b21, b22 = (w_ref[pl.ds(rr, 16), pl.ds(cc, w)].astype(f32)
                                  for rr in (r, kh + r) for cc in (c0, nh + c0))
            if transposed:
                b12, b21 = b21, b12
            r2 = pl.multiple_of(row0 + (start + u) * 8, 8)
            tok = None
            for n, t in enumerate((b11 + b22, b11, b12 - b22, b21 - b11, b22, b11 + b12, b21 + b22)):
                t = _pack(t)
                c_ref[n, pl.ds(r2, 8), pl.ds(c0, w)] = t
                for l0 in range(0, w, 128):
                    tok = t[:, l0:l0 + 128] if tok is None else tok | t[:, l0:l0 + 128]
            return pltpu.bitcast(tok, f32)
        return run
    return [job(u, c0, min(256, nh - c0)) for u in range(per) for c0 in range(0, nh, 256)]


def _strassen(ac, c_ref, cw, z):
    out = [[], [], [], []]
    for c0 in range(0, c_ref.shape[2], cw):
        def m(i):
            return jnp.dot(ac[i], _unpack(c_ref[i + z, :, c0:c0 + cw]), preferred_element_type=f32)
        m2, m4 = m(1), m(3)
        out[2].append(m2 + m4)
        m1 = m(0)
        t11, t22 = m1 + m4, m1 - m2
        m3 = m(2)
        t22 = t22 + m3
        m5 = m(4)
        out[1].append(m3 + m5)
        out[0].append(t11 - m5 + m(6))
        out[3].append(t22 + m(5))
    return jnp.concatenate(out[0] + out[1], axis=1), jnp.concatenate(out[2] + out[3], axis=1)


def _strassen_t(ac, c_ref, row0, z):
    def m(i):
        return lax.dot_general(_unpack(c_ref[i + z, row0:row0 + HD // 2, :]), ac[i], NT_DIMS,
                               preferred_element_type=f32)
    m2, m4 = m(1), m(3)
    c21 = m2 + m4
    m1, m3 = m(0), m(2)
    t11, t22 = m1 + m4, m1 - m2 + m3
    m5 = m(4)
    c12 = m3 + m5
    c11 = t11 - m5 + m(6)
    c22 = t22 + m(5)
    return jnp.concatenate([c11, c12], axis=0), jnp.concatenate([c21, c22], axis=0)


def _plan():
    def groups(first, n):
        out = [(first + i, 32) for i in range(int(n))]
        return out + [(first + int(n), 16)] * (n != int(n))
    subs = [groups(0, m) + groups(4, n) for m, n in zip(NP0, NS)]
    nrows = sum(NC * 16 - sum(r // 8 for _, r in x) for x in subs)
    pieces = [(b, c, a, j) for b in range(NB) for c, r in subs[b] for a in range(r // 16) for j in range(4)]
    wts = [0.0 if r < START else W1 if r < Z1 else W2 if r >= nrows - Z2 else 1.0 for r in range(nrows)]
    pos = {}
    row, cum = 0, 0.0
    for k, pc in enumerate(pieces):
        while cum + wts[row] <= (k + 0.5) * sum(wts) / len(pieces):
            cum += wts[row]
            row += 1
        pos[pc] = row
    order = []
    row = 0
    for b in range(NB):
        mixed = list(subs[b])
        pure = [c for c in range(NC) if c not in dict(mixed)]
        while mixed or pure:
            if mixed and (not pure or row + (LAG - PVM) * RPS > pos[(b, mixed[0][0], mixed[0][1] // 16 - 1, 3)]):
                order.append((b,) + mixed.pop(0))
            else:
                order.append((b, pure.pop(0), 0))
            row += 16 - order[-1][2] // 8
    rows = [(i, r) for i, x in enumerate(order) for r in range(16 - x[2] // 8)]
    step_of = {x[:2]: i for i, x in enumerate(order)}
    attach = {}
    foreign = {(b, j): [] for b in range(NB) for j in range(4)}
    for (pb, c, a, j), p in pos.items():
        i, r = rows[p]
        assert step_of[(pb, c)] - NR + LAG < i <= step_of[(pb, c)] + LAG
        assert pb < NB - 1 or i >= LAG
        attach.setdefault((i, r, j), []).append((pb, c, a))
        if pb != order[i][0]:
            foreign[(pb, j)].append(c * 2 + a)
    return order, attach, foreign


def _kernel(x_hbm, wqkv_hbm, wo_hbm, w1_hbm, b1_hbm, w2_hbm, b2_hbm, o_hbm,
            x_ref, wqkv_ref, wo_ref, w1_ref, w2_ref, sem_x, sem_w, sem_o,
            xres, wqt, wvt, k_s, qt_s, vt_s, qf_s, kt_s, ot_s, qm_s, st_s, sc_s, zv_s, bias_s, z_s, *bufs):
    ring = bufs[:NR]
    kbs = bufs[NR:NR + 4]
    lacc = bufs[NR + 4:NR + 4 + NB]
    b1_ref, b2_ref, w1c, w2c, wkc, wqvc, wot = bufs[NR + 4 + NB:]

    def x_copy(r):
        rows = pl.ds(pl.multiple_of(r * TI, TI), TI)
        return pltpu.make_async_copy(x_hbm.at[rows], x_ref.at[rows], sem_x.at[r])

    def o_copy(r):
        rows = pl.ds(pl.multiple_of(r * TR, TR), TR)
        return pltpu.make_async_copy(x_ref.at[rows], o_hbm.at[rows], sem_o.at[r])
    b_copies = [pltpu.make_async_copy(b1_hbm, b1_ref.at[pl.ds(0, F)], sem_w.at[0]),
                pltpu.make_async_copy(b2_hbm, b2_ref.at[pl.ds(0, D)], sem_w.at[1])]
    qkv_copies = [pltpu.make_async_copy(wqkv_hbm.at[:, pl.ds(i * D, D)], wqkv_ref.at[i], sem_w.at[3 + i])
                  for i in range(3)]
    w_copies = [[], []]
    for src, dst in ((w1_hbm, w1_ref), (w2_hbm, w2_ref)):
        kh = src.shape[0] // 2
        cut = -(-(kh // 16) // 3) * 16
        for half in (0, kh):
            for stage, rows in enumerate((pl.ds(half, cut), pl.ds(half + cut, kh - cut))):
                sem = sem_w.at[6 + len(w_copies[0]) + len(w_copies[1])]
                w_copies[stage].append(pltpu.make_async_copy(src.at[rows], dst.at[rows], sem))
    w_copies[0].append(pltpu.make_async_copy(wo_hbm.at[pl.ds(0, HD)], wo_ref.at[pl.ds(0, HD)], sem_w.at[2]))
    w_copies[1].append(pltpu.make_async_copy(wo_hbm.at[pl.ds(HD, HD)], wo_ref.at[pl.ds(HD, HD)], sem_w.at[14]))
    x_copy(0).start()
    qkv_copies[1].start()

    qm_s[...] = jnp.zeros_like(qm_s)
    st_s[...] = jnp.zeros_like(st_s)
    zv_s[...] = jnp.zeros_like(zv_s)
    for buf in ring[NR - LAG:]:
        buf[...] = jnp.zeros_like(buf)
    lacc[NB - 1][...] = jnp.ones_like(lacc[NB - 1])
    for i in range(NZ):
        z_s[i] = 0

    def put_k(r0, k):
        kp = _pack(k)
        r2 = pl.multiple_of(r0 // 2, TR // 2)
        for g in range(4):
            k_s[g, pl.ds(r2, TR // 2), :] = kp[:, g * 128:(g + 1) * 128]
        kt = k.T.reshape(H, DH, TR)
        st_s[1] = jnp.maximum(st_s[1], jnp.sum(kt * kt, axis=1))
        return k[0:32]

    def put_qv(r0, q, v):
        q = q * QSCALE
        qt_s[:, pl.ds(r0, TR)] = _pack(q)
        q3 = q.reshape(H, DH, TR)
        qf_s[:, :, pl.ds(r0, TR)] = q3
        vt_s[:, pl.ds(r0, TR)] = _pack(v)
        st_s[0] = jnp.maximum(st_s[0], jnp.sum(q3 * q3, axis=1))
        st_s[2] = jnp.maximum(st_s[2], jnp.max(jnp.abs(v).reshape(DH, H, TR), axis=0))

    def put_kt(r, heads):
        kt_s[r] = jnp.concatenate(heads, axis=0).T.reshape(H, DH, 128)

    def proj_k(r0, xb):
        return put_k(r0, jnp.dot(xb, wqkv_ref[1], preferred_element_type=f32))

    def proj_qv(r0, xb, jobs=(), never=None):
        out = []
        for n, w in enumerate((wqt, wvt)):
            y = lax.dot_general(w[...], xb, NT_DIMS, preferred_element_type=f32)
            mine = jobs[n::2]
            if mine:
                step = D // len(mine) // 8 * 8
                parts = []
                for i, run in enumerate(mine):
                    parts.append(jnp.where(never, run(), y[i * step:i * step + 8]))
                    parts.append(y[i * step + 8:(i + 1) * step if i + 1 < len(mine) else D])
                y = jnp.concatenate(parts, axis=0)
            out.append(y)
        put_qv(r0, *out)

    def proj_pair(r1, x1, r2, x2, z):
        ac = _lhs_combos(_ln(x1), _ln(x2))
        k1, k2 = _strassen(ac, wkc, 128, z)
        kh = [put_k(r1, k1), put_k(r2, k2)]
        q1, q2 = _strassen_t(ac, wqvc, 0, z)
        v1, v2 = _strassen_t(ac, wqvc, HD // 2, z)
        put_qv(r1, q1, v1)
        put_qv(r2, q2, v2)
        return kh

    def prep(h, t):
        for d in range(DH):
            row = jnp.broadcast_to(kt_s[t, h, pl.ds(d, 1), :], (128, 128))
            kbs[t][0, d, pl.ds(0, 128), :] = row.T

    def load_x(r0):
        x = x_ref[pl.ds(r0, TR), :].astype(f32)
        xres[pl.ds(r0, TR), :] = x
        return _ln(x).astype(bf16)

    def first(r, c):
        @pl.when(r == 2)
        def _():
            for cp in w_copies[1]:
                cp.wait()
        x_copy(r).wait()
        prep(0, 0)
        never = zv_s[z_s[0]] != 0
        jobs = (_rhs_jobs(w1_ref, w1c, r - 1) + _rhs_jobs(w2_ref, w2c, r - 1)
                + _rhs_jobs(wqkv_ref.at[1], wkc, r - 1) + _rhs_jobs(wqt, wqvc, r - 1, True)
                + _rhs_jobs(wvt, wqvc, r - 1, True, HD // 2))

        def wo_job(u):
            def run():
                c0 = pl.multiple_of((r - 1 + u) * 128, 128)
                y = wo_ref[pl.ds(c0, 128), :].astype(f32).T
                wot[:, pl.ds(c0, 128)] = y.astype(bf16)
                return jnp.max(y.reshape(D // 8, 8, 128), axis=0)
            return run
        jobs = jobs[:30] + [wo_job(0)] + jobs[30:50] + [wo_job(1)] + jobs[50:]
        kh = []
        for t in range(NT):
            r0 = pl.multiple_of(r * TI + t * TR, TR)
            xb = load_x(r0)
            kh.append(proj_k(r0, xb))
            proj_qv(r0, xb, jobs[t::NT], never)
        put_kt(r, kh)
        return c

    x_copy(0).wait()
    qkv_copies[0].start()
    qkv_copies[2].start()
    xbs = [load_x(0)]
    qkv_copies[1].wait()
    x_copy(1).start()
    for cp in w_copies[0]:
        cp.start()
    xbs += [load_x(t * TR) for t in range(1, NT)]
    kh0 = [proj_k(t * TR, xbs[t]) for t in range(NT - 1)]
    qkv_copies[0].wait()
    qkv_copies[2].wait()
    x_copy(2).start()
    for cp in w_copies[1]:
        cp.start()
    wqt[...] = wqkv_ref[0].astype(f32).T.astype(bf16)
    wvt[...] = wqkv_ref[2].astype(f32).T.astype(bf16)
    kh0.append(proj_k((NT - 1) * TR, xbs[NT - 1]))
    for t in range(NT):
        proj_qv(t * TR, xbs[t])
    put_kt(0, kh0)
    for cp in w_copies[0]:
        cp.wait()
    x_copy(3).start()
    for cp in b_copies:
        cp.start()
    lax.fori_loop(1, S // TI, first, 0)

    def set_q(h):
        moff = pl.multiple_of((h % 8) * 8, 8)
        poff = pl.multiple_of(((h + 7) % 8) * 8, 8)
        qm_s[0, pl.ds(poff, 8), :] = jnp.zeros((8, S), u32)
        qm_s[0, pl.ds(moff, 8), :] = qt_s[pl.ds(pl.multiple_of(h * 8, 8), 8), :]

    order, attach, foreign = _plan()
    no = len(order)
    bufof = {x[:2]: ring[i % NR] for i, x in enumerate(order)}

    def head_fast(h, o_prev, main=True):
        g = h // 8
        hp = jnp.maximum(h - 1, 0)
        hpo = jnp.where(h > 0, h - 1, H)
        if main:
            for t in sorted({x[1] // 4 for x in order if x[2]} - {0}):
                prep(h, t)
        zc = [0]

        def zero():
            zc[0] += 1
            return z_s[zc[0] - 1]
        never = zv_s[zero()] != 0
        o = [None] * NB + [o_prev]
        l = [[None] * 4 for _ in range(NB)]

        def do_vpu(b, c, a, j):
            t, sb = divmod(c, 4)
            acc = [None, None]
            z = zero()
            hq = h + z
            for d in range(DH):
                kbd = kbs[t][z, d, pl.ds(sb * 32 + a * 16, 16), :]
                qd = qf_s[hq, pl.ds(d, 1), pl.ds(b * TQ + j * 128, 128)]
                tt = kbd * qd
                acc[d % 2] = tt if acc[d % 2] is None else acc[d % 2] + tt
            p = jnp.exp2(acc[0] + acc[1])
            bufof[(b, c)][0, j, pl.ds(a * 16, 16), :] = p.astype(bf16)
            return p[0:8] + p[8:16]

        def do_qk(i):
            b, ci, r0 = order[i]
            z = zero()
            kc = _unpack(k_s[g + z, pl.ds((ci * KC + r0) // 2, (KC - r0) // 2), :])
            qm = _unpack(qm_s[z, :, pl.ds(b * TQ, TQ)])
            p = jnp.exp2(jnp.dot(kc, qm, preferred_element_type=f32))
            nr = (KC - r0) // 8
            p3 = p.reshape(nr, 8, TQ)
            nxt = [0] * 4
            for j in range(4):
                bufof[(b, ci)][0, j, pl.ds(r0, KC - r0), :] = p[:, 128 * j:128 * j + 128].astype(bf16)

            def flush(j, upto):
                if upto > nxt[j]:
                    seg = p3[nxt[j]:upto, :, 128 * j:128 * j + 128]
                    if l[b][j] is not None:
                        seg = jnp.concatenate([l[b][j][None], seg], axis=0)
                    l[b][j] = jnp.sum(seg, axis=0)
                    nxt[j] = upto
            for r in range(nr):
                for j in range(4):
                    for pb, c, a in attach.get((i, r, j), []):
                        flush(j, r + 1)
                        ps = do_vpu(pb, c, a, j)
                        if pb != b:
                            lacc[pb][0, 1 + c * 2 + a, :, pl.ds(j * 128, 128)] = ps
                            l[b][j] = jnp.where(never, ps, l[b][j])
                        else:
                            l[b][j] = l[b][j] + ps
            for j in range(4):
                flush(j, nr)
            if i == no - 1 or order[i + 1][0] != b:
                lacc[b][0, 0] = jnp.concatenate(l[b], axis=-1)
        done = [0] * NB + [NC - LAG]

        def do_pv(i):
            prev = i < 0
            b, ci, _ = order[i % no]
            ob = NB if prev else b
            z = zero()
            h8 = pl.multiple_of((hp if prev else h) * 8, 8)
            vt = _unpack(vt_s[pl.ds(h8, 8), pl.ds(ci * KC, KC)])
            words = bufof[(b, ci)].bitcast(u32)
            p = jnp.concatenate([_unpack(words[z, j, pl.ds(0, KC // 2), :]) for j in range(4)], axis=1)
            pv = jnp.dot(vt, p, preferred_element_type=f32)
            o[ob] = pv if o[ob] is None else o[ob] + pv
            done[ob] += 1
            if done[ob] == NC:
                cols = []
                for j in range(4):
                    v = lacc[b][z, 0, :, pl.ds(j * 128, 128)]
                    for sub in foreign[(b, j)]:
                        v = v + lacc[b][z, 1 + sub, :, pl.ds(j * 128, 128)]
                    cols.append(v)
                lsum = jnp.sum(jnp.concatenate(cols, axis=-1), axis=0, keepdims=True)
                hoff = pl.multiple_of((hpo if prev else h) * DH, DH)
                ot_s[pl.ds(hoff, DH), pl.ds(b * TQ, TQ)] = o[ob] * _recip(lsum)
        for i in range(no if main else LAG):
            if main:
                do_qk(i)
            do_pv(i - LAG)
        assert zc[0] <= NZ
        if main:
            set_q((h + 1) % H)
            prep((h + 1) % H, 0)
            return o[NB - 1]

    def head_safe(h, c):
        g = h // 8
        hoff = pl.multiple_of(h * DH, DH)
        h8 = pl.multiple_of(h * 8, 8)
        set_q(h)

        def blk(b, c2):
            q0 = pl.multiple_of(b * TQ, TQ)
            qm = _unpack(qm_s[0, :, pl.ds(q0, TQ)])

            def scores(ci, m):
                kc = _unpack(k_s[g, pl.ds(pl.multiple_of(ci * 128, 128), 128), :])
                s = jnp.dot(kc, qm, preferred_element_type=f32)
                sc_s[pl.ds(pl.multiple_of(ci * 256, 256), 256), :] = s
                return jnp.maximum(m, jnp.max(s.reshape(32, 8, TQ), axis=0))
            m = lax.fori_loop(0, S // 256, scores, jnp.full((8, TQ), -jnp.inf, f32))
            m = jnp.max(m, axis=0, keepdims=True)

            def accum(ci, lo):
                c0 = pl.multiple_of(ci * 256, 256)
                p = jnp.exp2(sc_s[pl.ds(c0, 256), :] - m)
                vt = _unpack(vt_s[pl.ds(h8, 8), pl.ds(c0, 256)])
                return (lo[0] + jnp.sum(p.reshape(32, 8, TQ), axis=0),
                        lo[1] + jnp.dot(vt, p.astype(bf16), preferred_element_type=f32))
            l, o = lax.fori_loop(0, S // 256, accum, (jnp.zeros((8, TQ), f32), jnp.zeros((DH, TQ), f32)))
            ot_s[pl.ds(hoff, DH), pl.ds(q0, TQ)] = o * (1.0 / jnp.sum(l, axis=0, keepdims=True))
            return c2
        lax.fori_loop(0, NB, blk, 0)
        return c

    def attention():
        qn = jnp.max(st_s[0], axis=1, keepdims=True)
        kn = jnp.max(st_s[1], axis=1, keepdims=True)
        bound2 = jnp.max(qn * kn) * 1.05
        vmax = jnp.max(st_s[2])
        st_s[...] = jnp.zeros_like(st_s)
        ok = jnp.logical_and(bound2 <= SAFE_LOG2 * SAFE_LOG2,
                             jnp.logical_and(vmax <= 2.0 ** 40, vmax >= 2.0 ** -30))

        @pl.when(ok)
        def _():
            set_q(0)
            o_last = lax.fori_loop(0, H, head_fast, jnp.zeros((DH, TQ), f32))
            head_fast(H, o_last, main=False)

        @pl.when(jnp.logical_not(ok))
        def _():
            lax.fori_loop(0, H, head_safe, 0)

    def dense(last):
        def body(r, c):
            r0s = [pl.multiple_of(r * TI + t * TR, TR) for t in range(NT)]
            if not last:
                prep(0, 0)
            xs = []
            for t, r0 in enumerate(r0s):
                ot = ot_s[pl.ds(0, D), pl.ds(r0, TR)]
                if t == 0:
                    a = jnp.dot(wot[...], ot.astype(bf16), preferred_element_type=f32)
                    a = jnp.concatenate([a[:HD].T, a[HD:].T], axis=1)
                else:
                    a = jnp.dot(ot.T.astype(bf16), wo_ref[...], preferred_element_type=f32)
                xs.append(xres[pl.ds(r0, TR), :] + a)
            hs = []
            for t in range(0, NT, 2):
                h1, h2 = _strassen(_lhs_combos(_ln(xs[t]), _ln(xs[t + 1])), w1c, 128, z_s[t])
                hs.append(_lhs_combos(_gelu(h1 + bias_s[0:1, 0:F]), _gelu(h2 + bias_s[0:1, 0:F])))
            ds = []
            for t, hc in enumerate(hs):
                ds += _strassen(hc, w2c, 256, z_s[t])
            ys = []
            for t in range(NT):
                ys.append(xs[t] + ds[t] + bias_s[1:2, 0:D])
                if last:
                    x_ref[pl.ds(r0s[t], TR), :] = ys[t].astype(bf16)
                    o_copy(r * NT + t).start()
            if not last:
                for r0, x in zip(r0s, ys):
                    xres[pl.ds(r0, TR), :] = x
                kh = []
                for t in range(0, NT, 2):
                    kh += proj_pair(r0s[t], ys[t], r0s[t + 1], ys[t + 1], z_s[t])
                put_kt(r, kh)
            return c
        lax.fori_loop(0, S // TI, body, 0)

    def layer(i, c):
        attention()

        @pl.when(i == 0)
        def _():
            for cp in b_copies:
                cp.wait()
            bias_s[0:1, 0:F] = b1_ref[pl.ds(0, F)].astype(f32)[None, :]
            bias_s[1:2, 0:D] = b2_ref[pl.ds(0, D)].astype(f32)[None, :]
            dense(False)

        @pl.when(i == 1)
        def _():
            dense(True)
        return c
    lax.fori_loop(0, 2, layer, 0)
    for r in range(S // TR):
        o_copy(r).wait()


@jax.jit
def pallas_interleave_layers__mha_block__dense_activation_gelu__prompt_kernel(A_x, A_wqkv, A_wo, B_x, B_w1, B_b1, B_w2, B_b2):
    hbm = pl.BlockSpec(memory_space=pl.ANY)
    out = pl.pallas_call(
        _kernel,
        out_shape=jax.ShapeDtypeStruct((S, D), bf16),
        in_specs=[hbm] * 7,
        out_specs=hbm,
        scratch_shapes=[
            pltpu.VMEM((S, D), bf16),
            pltpu.VMEM((3, D, D), bf16),
            pltpu.VMEM((D, D), bf16),
            pltpu.VMEM((D, F), bf16),
            pltpu.VMEM((F, D), bf16),
            pltpu.SemaphoreType.DMA((S // TI,)),
            pltpu.SemaphoreType.DMA((15,)),
            pltpu.SemaphoreType.DMA((S // TR,)),
            pltpu.VMEM((S, D), f32),
            pltpu.VMEM((D, D), bf16),
            pltpu.VMEM((D, D), bf16),
            pltpu.VMEM((4, S // 2, 128), u32),
            pltpu.VMEM((D // 2, S), u32),
            pltpu.VMEM((D // 2, S), u32),
            pltpu.VMEM((H, DH, S), f32),
            pltpu.VMEM((4, H, DH, 128), f32),
            pltpu.VMEM((D + DH, S), f32),
            pltpu.VMEM((1, 64, S), u32),
            pltpu.VMEM((3, H, TR), f32),
            pltpu.VMEM((S, TQ), f32),
            pltpu.VMEM((4, 8, 128), jnp.int32),
            pltpu.VMEM((8, 2048), f32),
            pltpu.SMEM((NZ,), jnp.int32),
        ] + [pltpu.VMEM((1, 4, KC + RPAD, 128), bf16) for _ in range(NR)]
          + [pltpu.VMEM((1, DH, 128 + KPAD, 128), f32) for _ in range(4)]
          + [pltpu.VMEM((1, NL, 8, TQ), f32) for _ in range(NB)]
          + [pltpu.VMEM((8192,), bf16), pltpu.VMEM((8192,), bf16),
             pltpu.VMEM((7, HD // 2, FH), u32), pltpu.VMEM((7, FH // 2, HD), u32),
             pltpu.VMEM((7, HD // 2, HD), u32), pltpu.VMEM((7, HD, HD), u32),
             pltpu.VMEM((D, D), bf16)],
        compiler_params=pltpu.CompilerParams(vmem_limit_bytes=100 * 2 ** 20),
    )(A_x.reshape(S, D), A_wqkv, A_wo, B_w1, B_b1, B_w2, B_b2)
    return out.reshape(1, S, D)
```

```python
import jax
import jax.numpy as jnp
from jax import lax
import jax.experimental.pallas as pl
import jax.experimental.pallas.tpu as pltpu

S, D, H, DH, F = 2048, 512, 32, 16, 1792
TR = 128
NT = 4
TI = NT * TR
TQ = 512
KC = 128
NB = S // TQ
NC = S // KC
HD = D // 2
FH = F // 2

LAG = 4
NR = 16
NP0 = (3.5, 0, 0, 0)
NS = (5, 10, 10, 9)
START = 8
PVM = 2
RPS = 14
W1 = 0.9
Z1 = 170
W2 = 0.95
Z2 = 90
KPAD = 8
RPAD = 16
NL = 36
NZ = 600

QSCALE = (DH ** -0.5) * 1.4426950408889634
SAFE_LOG2 = 60.0
bf16 = jnp.bfloat16
f32 = jnp.float32
u32 = jnp.uint32
NT_DIMS = (((1,), (1,)), ((), ()))


def _ln(x):
    m = jnp.mean(x, axis=-1, keepdims=True)
    xc = x - m
    v = jnp.mean(xc * xc, axis=-1, keepdims=True)
    return xc * lax.rsqrt(v + 1e-5)


def _gelu(x):
    c = 0.7978845608028654
    return 0.5 * x * (1.0 + jnp.tanh(c * (x + 0.044715 * (x * x * x))))


def _recip(x):
    r = pl.reciprocal(x, approx=True)
    return r * (2.0 - x * r)


def _pack(x):
    return pltpu.bitcast(x.astype(bf16), u32)


def _unpack(x):
    return pltpu.bitcast(x, bf16)


def _lhs_combos(a1, a2):
    kh = a1.shape[1] // 2
    a11, a12, a21, a22 = a1[:, :kh], a1[:, kh:], a2[:, :kh], a2[:, kh:]
    return [t.astype(bf16) for t in (a11 + a22, a21 + a22, a11, a22, a11 + a12, a21 - a11, a12 - a22)]


def _rhs_jobs(w_ref, c_ref, part, transposed=False, row0=0):
    kh, nh = w_ref.shape[0] // 2, w_ref.shape[1] // 2
    units = kh // 16
    per = -(-units // 3)
    start = jnp.minimum(part * per, units - per)

    def job(u, c0, w):
        def run():
            r = pl.multiple_of((start + u) * 16, 16)
            b11, b12, b21, b22 = (w_ref[pl.ds(rr, 16), pl.ds(cc, w)].astype(f32)
                                  for rr in (r, kh + r) for cc in (c0, nh + c0))
            if transposed:
                b12, b21 = b21, b12
            r2 = pl.multiple_of(row0 + (start + u) * 8, 8)
            tok = None
            for n, t in enumerate((b11 + b22, b11, b12 - b22, b21 - b11, b22, b11 + b12, b21 + b22)):
                t = _pack(t)
                c_ref[n, pl.ds(r2, 8), pl.ds(c0, w)] = t
                for l0 in range(0, w, 128):
                    tok = t[:, l0:l0 + 128] if tok is None else tok | t[:, l0:l0 + 128]
            return pltpu.bitcast(tok, f32)
        return run
    return [job(u, c0, min(256, nh - c0)) for u in range(per) for c0 in range(0, nh, 256)]


def _strassen(ac, c_ref, cw, z):
    out = [[], [], [], []]
    for c0 in range(0, c_ref.shape[2], cw):
        def m(i):
            return jnp.dot(ac[i], _unpack(c_ref[i + z, :, c0:c0 + cw]), preferred_element_type=f32)
        m2, m4 = m(1), m(3)
        out[2].append(m2 + m4)
        m1 = m(0)
        t11, t22 = m1 + m4, m1 - m2
        m3 = m(2)
        t22 = t22 + m3
        m5 = m(4)
        out[1].append(m3 + m5)
        out[0].append(t11 - m5 + m(6))
        out[3].append(t22 + m(5))
    return jnp.concatenate(out[0] + out[1], axis=1), jnp.concatenate(out[2] + out[3], axis=1)


def _strassen_t(ac, c_ref, row0, z):
    def m(i):
        return lax.dot_general(_unpack(c_ref[i + z, row0:row0 + HD // 2, :]), ac[i], NT_DIMS,
                               preferred_element_type=f32)
    m2, m4 = m(1), m(3)
    c21 = m2 + m4
    m1, m3 = m(0), m(2)
    t11, t22 = m1 + m4, m1 - m2 + m3
    m5 = m(4)
    c12 = m3 + m5
    c11 = t11 - m5 + m(6)
    c22 = t22 + m(5)
    return jnp.concatenate([c11, c12], axis=0), jnp.concatenate([c21, c22], axis=0)


def _plan():
    def groups(first, n):
        out = [(first + i, 32) for i in range(int(n))]
        return out + [(first + int(n), 16)] * (n != int(n))
    subs = [groups(0, m) + groups(4, n) for m, n in zip(NP0, NS)]
    nrows = sum(NC * 16 - sum(r // 8 for _, r in x) for x in subs)
    pieces = [(b, c, a, j) for b in range(NB) for c, r in subs[b] for a in range(r // 16) for j in range(4)]
    wts = [0.0 if r < START else W1 if r < Z1 else W2 if r >= nrows - Z2 else 1.0 for r in range(nrows)]
    pos = {}
    row, cum = 0, 0.0
    for k, pc in enumerate(pieces):
        while cum + wts[row] <= (k + 0.5) * sum(wts) / len(pieces):
            cum += wts[row]
            row += 1
        pos[pc] = row
    order = []
    row = 0
    for b in range(NB):
        mixed = list(subs[b])
        pure = [c for c in range(NC) if c not in dict(mixed)]
        while mixed or pure:
            gap = NB * NC - LAG - len(order)
            keep = 1 if b == NB - 1 and gap > 0 else 0
            if mixed and gap != 0 and (len(pure) <= keep or row + (LAG - PVM + (gap == 1)) * RPS
                                       > pos[(b, mixed[0][0], mixed[0][1] // 16 - 1, 3)]):
                order.append((b,) + mixed.pop(0))
            else:
                order.append((b, pure.pop(0), 0))
            row += 16 - order[-1][2] // 8
    rows = [(i, r) for i, x in enumerate(order) for r in range(16 - x[2] // 8)]
    step_of = {x[:2]: i for i, x in enumerate(order)}
    attach = {}
    foreign = {(b, j): [] for b in range(NB) for j in range(4)}
    for (pb, c, a, j), p in pos.items():
        i, r = rows[p]
        assert step_of[(pb, c)] - NR + LAG < i <= step_of[(pb, c)] + LAG
        assert pb < NB - 1 or i >= LAG
        attach.setdefault((i, r, j), []).append((pb, c, a))
        if pb != order[i][0]:
            foreign[(pb, j)].append(c * 2 + a)
    return order, attach, foreign


def _kernel(x_hbm, wqkv_hbm, wo_hbm, w1_hbm, b1_hbm, w2_hbm, b2_hbm, o_hbm,
            x_ref, wqkv_ref, wo_ref, w1_ref, w2_ref, sem_x, sem_w, sem_o,
            xres, wqt, wvt, k_s, qt_s, vt_s, qf_s, kt_s, ot_s, st_s, sc_s, zv_s, bias_s, z_s, *bufs):
    ring = bufs[:NR]
    kbs = bufs[NR:NR + 4]
    lacc = bufs[NR + 4:NR + 4 + NB]
    b1_ref, b2_ref, w1c, w2c, wkc, wqvc, wot = bufs[NR + 4 + NB:]

    def x_copy(r):
        rows = pl.ds(pl.multiple_of(r * TI, TI), TI)
        return pltpu.make_async_copy(x_hbm.at[rows], x_ref.at[r], sem_x.at[r])

    def o_copy(r, t):
        rows = pl.ds(pl.multiple_of(r * TI + t * TR, TR), TR)
        return pltpu.make_async_copy(x_ref.at[r, pl.ds(t * TR, TR)], o_hbm.at[rows], sem_o.at[r * NT + t])
    b_copies = [pltpu.make_async_copy(b1_hbm, b1_ref.at[pl.ds(0, F)], sem_w.at[0]),
                pltpu.make_async_copy(b2_hbm, b2_ref.at[pl.ds(0, D)], sem_w.at[1])]
    qkv_copies = [pltpu.make_async_copy(wqkv_hbm.at[:, pl.ds(i * D, D)], wqkv_ref.at[i], sem_w.at[3 + i])
                  for i in range(3)]
    w_copies = [[], []]
    for src, dst in ((w1_hbm, w1_ref), (w2_hbm, w2_ref)):
        kh = src.shape[0] // 2
        cut = -(-(kh // 16) // 3) * 16
        for half in (0, kh):
            for stage, rows in enumerate((pl.ds(half, cut), pl.ds(half + cut, kh - cut))):
                sem = sem_w.at[6 + len(w_copies[0]) + len(w_copies[1])]
                w_copies[stage].append(pltpu.make_async_copy(src.at[rows], dst.at[rows], sem))
    w_copies[0].append(pltpu.make_async_copy(wo_hbm.at[pl.ds(0, HD)], wo_ref.at[pl.ds(0, HD)], sem_w.at[2]))
    w_copies[1].append(pltpu.make_async_copy(wo_hbm.at[pl.ds(HD, HD)], wo_ref.at[pl.ds(HD, HD)], sem_w.at[14]))
    x_copy(0).start()
    qkv_copies[1].start()

    st_s[...] = jnp.zeros_like(st_s)
    zv_s[...] = jnp.zeros_like(zv_s)
    for buf in ring[NR - LAG:]:
        buf[...] = jnp.zeros_like(buf)
    lacc[NB - 1][...] = jnp.ones_like(lacc[NB - 1])
    for i in range(NZ):
        z_s[i] = 0

    def put_k(r, t, k):
        kp = _pack(k)
        for g in range(4):
            kg = kp[:, g * 128:(g + 1) * 128]
            for sl in range(8):
                k_s[g * 8 + sl, r, pl.ds(t * TR // 2, TR // 2), :] = pltpu.roll(kg, 128 - DH * sl, 1) if sl else kg
        kt = k.T.reshape(H, DH, TR)
        st_s[1] = jnp.maximum(st_s[1], jnp.sum(kt * kt, axis=1))
        return k[0:32]

    def put_qv(r, t, q, v):
        cols = pl.ds(t * TR, TR)
        q = q * QSCALE
        qt_s[r, :, :, cols] = _pack(q).reshape(H, 8, TR)
        q3 = q.reshape(H, DH, TR)
        qf_s[r, :, :, cols] = q3
        vt_s[r, :, :, cols] = _pack(v).reshape(H, 8, TR)
        st_s[0] = jnp.maximum(st_s[0], jnp.sum(q3 * q3, axis=1))
        st_s[2] = jnp.maximum(st_s[2], jnp.max(jnp.abs(v).reshape(DH, H, TR), axis=0))

    def put_kt(r, heads):
        kt_s[r] = jnp.concatenate(heads, axis=0).T.reshape(H, DH, 128)

    def proj_k(r, t, xb):
        return put_k(r, t, jnp.dot(xb, wqkv_ref[1], preferred_element_type=f32))

    def proj_qv(r, t, xb, jobs=(), never=None):
        out = []
        for n, w in enumerate((wqt, wvt)):
            y = lax.dot_general(w[...], xb, NT_DIMS, preferred_element_type=f32)
            mine = jobs[n::2]
            if mine:
                step = D // len(mine) // 8 * 8
                parts = []
                for i, run in enumerate(mine):
                    parts.append(jnp.where(never, run(), y[i * step:i * step + 8]))
                    parts.append(y[i * step + 8:(i + 1) * step if i + 1 < len(mine) else D])
                y = jnp.concatenate(parts, axis=0)
            out.append(y)
        put_qv(r, t, *out)

    def proj_pair(r, t, x1, x2, z):
        ac = _lhs_combos(_ln(x1), _ln(x2))
        k1, k2 = _strassen(ac, wkc, 128, z)
        kh = [put_k(r, t, k1), put_k(r, t + 1, k2)]
        q1, q2 = _strassen_t(ac, wqvc, 0, z)
        v1, v2 = _strassen_t(ac, wqvc, HD // 2, z)
        put_qv(r, t, q1, v1)
        put_qv(r, t + 1, q2, v2)
        return kh

    def prep(h, t):
        for d in range(DH):
            row = jnp.broadcast_to(kt_s[t, h, pl.ds(d, 1), :], (128, 128))
            kbs[t][0, d, pl.ds(0, 128), :] = row.T

    def load_x(r, t):
        x = x_ref[r, pl.ds(t * TR, TR), :].astype(f32)
        xres[r, pl.ds(t * TR, TR), :] = x
        return _ln(x).astype(bf16)

    def first(r, c):
        @pl.when(r == 2)
        def _():
            for cp in w_copies[1]:
                cp.wait()
        x_copy(r).wait()
        prep(0, 0)
        never = zv_s[z_s[0]] != 0
        jobs = (_rhs_jobs(w1_ref, w1c, r - 1) + _rhs_jobs(w2_ref, w2c, r - 1)
                + _rhs_jobs(wqkv_ref.at[1], wkc, r - 1) + _rhs_jobs(wqt, wqvc, r - 1, True)
                + _rhs_jobs(wvt, wqvc, r - 1, True, HD // 2))

        def wo_job(u):
            def run():
                c0 = pl.multiple_of((r - 1 + u) * 128, 128)
                y = wo_ref[pl.ds(c0, 128), :].astype(f32).T
                wot[:, pl.ds(c0, 128)] = y.astype(bf16)
                return jnp.max(y.reshape(D // 8, 8, 128), axis=0)
            return run
        jobs = jobs[:30] + [wo_job(0)] + jobs[30:50] + [wo_job(1)] + jobs[50:]
        kh = []
        for t in range(NT):
            xb = load_x(r, t)
            kh.append(proj_k(r, t, xb))
            proj_qv(r, t, xb, jobs[t::NT], never)
        put_kt(r, kh)
        return c

    x_copy(0).wait()
    qkv_copies[0].start()
    qkv_copies[2].start()
    xbs = [load_x(0, 0)]
    qkv_copies[1].wait()
    x_copy(1).start()
    for cp in w_copies[0]:
        cp.start()
    xbs += [load_x(0, t) for t in range(1, NT)]
    ks = [jnp.dot(xbs[t], wqkv_ref[1], preferred_element_type=f32) for t in range(NT - 1)]
    kh0 = [put_k(0, 0, ks[0])]
    qkv_copies[0].wait()
    qkv_copies[2].wait()
    x_copy(2).start()
    for cp in w_copies[1]:
        cp.start()
    wqt[...] = wqkv_ref[0].astype(f32).T.astype(bf16)
    wvt[...] = wqkv_ref[2].astype(f32).T.astype(bf16)
    kh0 += [put_k(0, t, ks[t]) for t in range(1, NT - 1)]
    kh0.append(proj_k(0, NT - 1, xbs[NT - 1]))
    for t in range(NT):
        proj_qv(0, t, xbs[t])
    put_kt(0, kh0)
    for cp in w_copies[0]:
        cp.wait()
    x_copy(3).start()
    for cp in b_copies:
        cp.start()
    lax.fori_loop(1, S // TI, first, 0)

    order, attach, foreign = _plan()
    no = len(order)
    bufof = {x[:2]: ring[i % NR] for i, x in enumerate(order)}

    def head_fast(h, o_prev, main=True):
        hp = jnp.maximum(h - 1, 0)
        hpo = jnp.where(h > 0, h - 1, H)
        if main:
            for t in sorted({x[1] // 4 for x in order if x[2]} - {0}):
                prep(h, t)
        zc = [0]

        def zero():
            zc[0] += 1
            return z_s[zc[0] - 1]
        never = zv_s[zero()] != 0
        o = [None] * NB + [o_prev]
        l = [[None] * 4 for _ in range(NB)]

        def do_vpu(b, c, a, j):
            t, sb = divmod(c, 4)
            acc = [None, None]
            z = zero()
            hq = h + z
            for d in range(DH):
                kbd = kbs[t][z, d, pl.ds(sb * 32 + a * 16, 16), :]
                qd = qf_s[b, hq, pl.ds(d, 1), pl.ds(j * 128, 128)]
                tt = kbd * qd
                acc[d % 2] = tt if acc[d % 2] is None else acc[d % 2] + tt
            p = jnp.exp2(acc[0] + acc[1])
            bufof[(b, c)][0, j, pl.ds(a * 16, 16), :] = p.astype(bf16)
            return p[0:8] + p[8:16]

        def do_qk(i):
            b, ci, r0 = order[i]
            z = zero()
            kc = _unpack(k_s[h + z, ci // NT, pl.ds((ci % NT * KC + r0) // 2, (KC - r0) // 2), pl.ds(0, DH)])
            qm = _unpack(qt_s[b, h + z])
            p = jnp.exp2(jnp.dot(kc, qm, preferred_element_type=f32))
            nr = (KC - r0) // 8
            p3 = p.reshape(nr, 8, TQ)
            nxt = [0] * 4
            for j in range(4):
                bufof[(b, ci)][0, j, pl.ds(r0, KC - r0), :] = p[:, 128 * j:128 * j + 128].astype(bf16)

            def flush(j, upto):
                if upto > nxt[j]:
                    seg = p3[nxt[j]:upto, :, 128 * j:128 * j + 128]
                    if l[b][j] is not None:
                        seg = jnp.concatenate([l[b][j][None], seg], axis=0)
                    l[b][j] = jnp.sum(seg, axis=0)
                    nxt[j] = upto
            for r in range(nr):
                for j in range(4):
                    for pb, c, a in attach.get((i, r, j), []):
                        flush(j, r + 1)
                        ps = do_vpu(pb, c, a, j)
                        if pb != b:
                            lacc[pb][0, 1 + c * 2 + a, :, pl.ds(j * 128, 128)] = ps
                            l[b][j] = jnp.where(never, ps, l[b][j])
                        else:
                            l[b][j] = l[b][j] + ps
            for j in range(4):
                flush(j, nr)
            if i == no - 1 or order[i + 1][0] != b:
                lacc[b][0, 0] = jnp.concatenate(l[b], axis=-1)
        done = [0] * NB + [NC - LAG]

        def do_pv(i):
            prev = i < 0
            b, ci, _ = order[i % no]
            ob = NB if prev else b
            z = zero()
            vt = _unpack(vt_s[ci // NT, hp if prev else h, :, pl.ds(ci % NT * KC, KC)])
            words = bufof[(b, ci)].bitcast(u32)
            p = jnp.concatenate([_unpack(words[z, j, pl.ds(0, KC // 2), :]) for j in range(4)], axis=1)
            pv = jnp.dot(vt, p, preferred_element_type=f32)
            o[ob] = pv if o[ob] is None else o[ob] + pv
            done[ob] += 1
            if done[ob] == NC:
                cols = []
                for j in range(4):
                    v = lacc[b][z, 0, :, pl.ds(j * 128, 128)]
                    for sub in foreign[(b, j)]:
                        v = v + lacc[b][z, 1 + sub, :, pl.ds(j * 128, 128)]
                    cols.append(v)
                lsum = jnp.sum(jnp.concatenate(cols, axis=-1), axis=0, keepdims=True)
                ot_s[b, hpo if prev else h] = o[ob] * _recip(lsum)
        for i in range(no if main else LAG):
            if main:
                do_qk(i)
            do_pv(i - LAG)
        assert zc[0] <= NZ
        if main:
            prep((h + 1) % H, 0)
            return o[NB - 1]

    def head_safe(h, c):
        def blk(b, c2):
            qm = _unpack(qt_s[b, h])

            def scores(ci, m):
                kc = _unpack(k_s[h, ci // 2, pl.ds(pl.multiple_of(ci % 2 * 128, 128), 128), pl.ds(0, DH)])
                s = jnp.dot(kc, qm, preferred_element_type=f32)
                sc_s[pl.ds(pl.multiple_of(ci * 256, 256), 256), :] = s
                return jnp.maximum(m, jnp.max(s.reshape(32, 8, TQ), axis=0))
            m = lax.fori_loop(0, S // 256, scores, jnp.full((8, TQ), -jnp.inf, f32))
            m = jnp.max(m, axis=0, keepdims=True)

            def accum(ci, lo):
                c0 = pl.multiple_of(ci * 256, 256)
                p = jnp.exp2(sc_s[pl.ds(c0, 256), :] - m)
                vt = _unpack(vt_s[ci // 2, h, :, pl.ds(pl.multiple_of(ci % 2 * 256, 256), 256)])
                return (lo[0] + jnp.sum(p.reshape(32, 8, TQ), axis=0),
                        lo[1] + jnp.dot(vt, p.astype(bf16), preferred_element_type=f32))
            l, o = lax.fori_loop(0, S // 256, accum, (jnp.zeros((8, TQ), f32), jnp.zeros((DH, TQ), f32)))
            ot_s[b, h] = o * (1.0 / jnp.sum(l, axis=0, keepdims=True))
            return c2
        lax.fori_loop(0, NB, blk, 0)
        return c

    def attention():
        qn = jnp.max(st_s[0], axis=1, keepdims=True)
        kn = jnp.max(st_s[1], axis=1, keepdims=True)
        bound2 = jnp.max(qn * kn) * 1.05
        vmax = jnp.max(st_s[2])
        st_s[...] = jnp.zeros_like(st_s)
        ok = jnp.logical_and(bound2 <= SAFE_LOG2 * SAFE_LOG2,
                             jnp.logical_and(vmax <= 2.0 ** 40, vmax >= 2.0 ** -30))

        @pl.when(ok)
        def _():
            o_last = lax.fori_loop(0, H, head_fast, jnp.zeros((DH, TQ), f32))
            head_fast(H, o_last, main=False)

        @pl.when(jnp.logical_not(ok))
        def _():
            lax.fori_loop(0, H, head_safe, 0)

    def dense(last):
        def body(r, c):
            if not last:
                prep(0, 0)
            xs = []
            for t in range(NT):
                ot = ot_s[r, pl.ds(0, H), :, pl.ds(t * TR, TR)].reshape(D, TR)
                if t == 0:
                    a = jnp.dot(wot[...], ot.astype(bf16), preferred_element_type=f32)
                    a = jnp.concatenate([a[:HD].T, a[HD:].T], axis=1)
                else:
                    a = jnp.dot(ot.T.astype(bf16), wo_ref[...], preferred_element_type=f32)
                xs.append(xres[r, pl.ds(t * TR, TR), :] + a)
            hs = []
            for t in range(0, NT, 2):
                h1, h2 = _strassen(_lhs_combos(_ln(xs[t]), _ln(xs[t + 1])), w1c, 128, z_s[t])
                hs.append(_lhs_combos(_gelu(h1 + bias_s[0:1, 0:F]), _gelu(h2 + bias_s[0:1, 0:F])))
            ds = []
            for t, hc in enumerate(hs):
                ds += _strassen(hc, w2c, 256, z_s[t])
            ys = []
            for t in range(NT):
                ys.append(xs[t] + ds[t] + bias_s[1:2, 0:D])
                if last:
                    x_ref[r, pl.ds(t * TR, TR), :] = ys[t].astype(bf16)
                    o_copy(r, t).start()
            if not last:
                for t in range(NT):
                    xres[r, pl.ds(t * TR, TR), :] = ys[t]
                kh = []
                for t in range(0, NT, 2):
                    kh += proj_pair(r, t, ys[t], ys[t + 1], z_s[t])
                put_kt(r, kh)
            return c
        lax.fori_loop(0, S // TI, body, 0)

    def layer(i, c):
        attention()

        @pl.when(i == 0)
        def _():
            for cp in b_copies:
                cp.wait()
            bias_s[0:1, 0:F] = b1_ref[pl.ds(0, F)].astype(f32)[None, :]
            bias_s[1:2, 0:D] = b2_ref[pl.ds(0, D)].astype(f32)[None, :]
            dense(False)

        @pl.when(i == 1)
        def _():
            dense(True)
        return c
    lax.fori_loop(0, 2, layer, 0)
    for r in range(NB):
        for t in range(NT):
            o_copy(r, t).wait()


@jax.jit
def pallas_interleave_layers__mha_block__dense_activation_gelu__prompt_kernel(A_x, A_wqkv, A_wo, B_x, B_w1, B_b1, B_w2, B_b2):
    hbm = pl.BlockSpec(memory_space=pl.ANY)
    out = pl.pallas_call(
        _kernel,
        out_shape=jax.ShapeDtypeStruct((S, D), bf16),
        in_specs=[hbm] * 7,
        out_specs=hbm,
        scratch_shapes=[
            pltpu.VMEM((NB, TI, D), bf16),
            pltpu.VMEM((3, D, D), bf16),
            pltpu.VMEM((D, D), bf16),
            pltpu.VMEM((D, F), bf16),
            pltpu.VMEM((F, D), bf16),
            pltpu.SemaphoreType.DMA((S // TI,)),
            pltpu.SemaphoreType.DMA((15,)),
            pltpu.SemaphoreType.DMA((S // TR,)),
            pltpu.VMEM((NB, TI, D), f32),
            pltpu.VMEM((D, D), bf16),
            pltpu.VMEM((D, D), bf16),
            pltpu.VMEM((H, S // TI, TI // 2, 128), u32),
            pltpu.VMEM((NB, H, 8, TQ), u32),
            pltpu.VMEM((NB, H, 8, TQ), u32),
            pltpu.VMEM((NB, H, DH, TQ), f32),
            pltpu.VMEM((4, H, DH, 128), f32),
            pltpu.VMEM((NB, H + 1, DH, TQ), f32),
            pltpu.VMEM((3, H, TR), f32),
            pltpu.VMEM((S, TQ), f32),
            pltpu.VMEM((4, 8, 128), jnp.int32),
            pltpu.VMEM((8, 2048), f32),
            pltpu.SMEM((NZ,), jnp.int32),
        ] + [pltpu.VMEM((1, 4, KC + RPAD, 128), bf16) for _ in range(NR)]
          + [pltpu.VMEM((1, DH, 128 + KPAD, 128), f32) for _ in range(4)]
          + [pltpu.VMEM((1, NL, 8, TQ), f32) for _ in range(NB)]
          + [pltpu.VMEM((8192,), bf16), pltpu.VMEM((8192,), bf16),
             pltpu.VMEM((7, HD // 2, FH), u32), pltpu.VMEM((7, FH // 2, HD), u32),
             pltpu.VMEM((7, HD // 2, HD), u32), pltpu.VMEM((7, HD, HD), u32),
             pltpu.VMEM((D, D), bf16)],
        compiler_params=pltpu.CompilerParams(vmem_limit_bytes=100 * 2 ** 20),
    )(A_x.reshape(S, D), A_wqkv, A_wo, B_w1, B_b1, B_w2, B_b2)
    return out.reshape(1, S, D)
```
